```python
import os as _os
_os.environ.setdefault("JAX_PLATFORMS", "cpu")
import jax
import jax.numpy as jnp

def _softmax(x, axis=-1):
    return jax.nn.softmax(x, axis=axis)
def _gelu(x):
    return jax.nn.gelu(x, approximate=True)
def _silu(x):
    return jax.nn.silu(x)
def _sigmoid(x):
    return jax.nn.sigmoid(x)
def _layernorm(x, axis=-1, eps=1e-5):
    m = jnp.mean(x, axis=axis, keepdims=True)
    v = jnp.var(x, axis=axis, keepdims=True)
    return (x - m) / jnp.sqrt(v + eps)
def _scatter_add(tgt, idx, src, axis=0):
    return tgt.at[idx].add(src)
def _segment_sum(src, seg, n):
    return jax.ops.segment_sum(src, seg, n)
class _Rng:
    def __init__(self, key):
        self._k = key
    def _next(self):
        self._k, sub = jax.random.split(self._k)
        return sub
    def normal(self, shape):
        return jax.random.normal(self._next(), shape, dtype=jnp.bfloat16)
    def randint(self, lo, hi, shape):
        return jax.random.randint(self._next(), shape, lo, hi, dtype=jnp.int32)
    def uniform(self, shape, lo=0.0, hi=1.0):
        return jax.random.uniform(self._next(), shape, jnp.bfloat16, lo, hi)
    def permutation(self, n):
        return jax.random.permutation(self._next(), n)


kernel_name = 'gated_mix__linear_kernel_hedgehog__mixer_s_mlp__prompt'

def setup_inputs():
    _rng = _Rng(jax.random.key(int.from_bytes(__import__("os").urandom(4), "little")))
    _w = (lambda a: (lambda t: t.astype(jnp.bfloat16) if jnp.issubdtype(t.dtype, jnp.floating) else t)(jnp.asarray(a)))
    def _A_setup():
        B, S, D, H = 1, 2048, 512, 32
        Dh = D // H
        return {
            "x": _w((lambda *s: _rng.normal(s) * 0.05)(B, S, D)),
            "wqkv": _w((lambda *s: _rng.normal(s) * 1.6)(D, 3 * D)),
            "w_phi": _w((lambda *s: _rng.normal(s) * 1.6)(H, Dh, Dh) * (Dh ** -0.5)),
            "wo": _w((lambda *s: _rng.normal(s) * 0.05)(D, D)),
        }
    _A_in = _A_setup()

    def _B_setup():
        B, S, D, F = 1, 2048, 512, 1376
        return {
            "x":  _w((lambda *s: _rng.normal(s) * 0.05)(B, S, D)),
            "w1": _w((lambda *s: _rng.normal(s) * 0.4)(D, D) * (D ** -0.5)),
            "w2": _w((lambda *s: _rng.normal(s) * 0.4)(D, D) * (D ** -0.5)),
            "w3": _w((lambda *s: _rng.normal(s) * 0.4)(D, F) * (D ** -0.5)),
            "w4": _w((lambda *s: _rng.normal(s) * 0.4)(F, D) * (F ** -0.5)),
        }
    _B_in = _B_setup()

    return {
        "A_x": _A_in["x"],
        "A_wqkv": _A_in["wqkv"],
        "A_w_phi": _A_in["w_phi"],
        "A_wo": _A_in["wo"],
        "B_x": _B_in["x"],
        "B_w1": _B_in["w1"],
        "B_w2": _B_in["w2"],
        "B_w3": _B_in["w3"],
        "B_w4": _B_in["w4"],
        "gate_w": _w((lambda *s: _rng.normal(s) * 0.05)(512) * 16.0),
    }

def reference(A_x, A_wqkv, A_w_phi, A_wo, B_x, B_w1, B_w2, B_w3, B_w4, gate_w):
    def _A_ref(x, wqkv, w_phi, wo):
        B, S, D = x.shape
        H = 32; Dh = D // H
        qkv = (lambda x, *d: x.transpose(*d))((x @ wqkv).reshape(B, S, 3, H, Dh), 2, 0, 3, 1, 4)
        q, k, v = qkv[0], qkv[1], qkv[2]
        pq = jnp.einsum("bhsd,hdf->bhsf", q, w_phi)
        pk = jnp.einsum("bhsd,hdf->bhsf", k, w_phi)
        phi_q = jnp.concatenate([_softmax(pq, axis=-1), _softmax(-pq, axis=-1)], axis=-1)
        phi_k = jnp.concatenate([_softmax(pk, axis=-1), _softmax(-pk, axis=-1)], axis=-1)
        kv = jnp.einsum("bhsf,bhsd->bhfd", phi_k, v)
        z  = jnp.einsum("bhsf->bhf", phi_k)
        num = jnp.einsum("bhqf,bhfd->bhqd", phi_q, kv)
        den = jnp.einsum("bhqf,bhf->bhq", phi_q, z)[..., None] + 1e-6
        o = num / den
        return (lambda x, *d: x.transpose(*d))(o, 0, 2, 1, 3).reshape(B, S, D) @ wo

    def _B_ref(x, w1, w2, w3, w4):
        B, S, D = x.shape
        h = _gelu(_layernorm(x, axis=-1) @ w1)
        c = D // 4
        g0 = jnp.pad(h[:, :, 0*c:1*c], ((0, 0), (1, 0), (0, 0)))[:, :S, :]
        g1 = jnp.pad(h[:, :, 1*c:2*c], ((0, 0), (0, 1), (0, 0)))[:, 1:, :]
        g2 = jnp.pad(h[:, :, 2*c:3*c], ((0, 0), (2, 0), (0, 0)))[:, :S, :]
        g3 = jnp.pad(h[:, :, 3*c:   ], ((0, 0), (0, 2), (0, 0)))[:, 2:, :]
        hs = jnp.concatenate([g0, g1, g2, g3], axis=-1) @ w2
        x1 = x + hs
        h2 = _gelu(_layernorm(x1, axis=-1) @ w3) @ w4
        return x1 + h2

    x = A_x
    g = _sigmoid((x * gate_w).sum(-1, keepdims=True))
    a = _A_ref(x, A_wqkv, A_w_phi, A_wo)
    b = _B_ref(x, B_w1, B_w2, B_w3, B_w4)
    return g * a + (1 - g) * b
```

```python
import functools
import math

import jax
import jax.numpy as jnp
import jax.experimental.pallas as pl
import jax.experimental.pallas.tpu as pltpu

S, D, H, DH, F = 2048, 512, 32, 16, 1376
TM1 = 512
TM2 = 512
NB1 = S // TM1
NB2 = S // TM2
LOG2E = math.log2(math.e)
GELU_C = math.sqrt(2.0 / math.pi)
BF = jnp.bfloat16
F32 = jnp.float32
NT = (((1,), (1,)), ((), ()))
G = 8


def _gelu(y):
    inner = y * (GELU_C + (GELU_C * 0.044715) * (y * y))
    hy = 0.5 * y
    return hy + hy * jnp.tanh(inner)


def _ln(xf):
    m = jnp.mean(xf, axis=-1, keepdims=True)
    xc = xf - m
    v = jnp.mean(xc * xc, axis=-1, keepdims=True)
    return xc * jax.lax.rsqrt(v + 1e-5)


def _fold4(op, t):
    return op(t, pltpu.roll(t, 4, 0))


def _dual_exp(p):
    p3 = p.reshape(8, 8, p.shape[-1])
    mx = _fold4(jnp.maximum, jnp.max(p3, axis=0))
    mn = _fold4(jnp.minimum, jnp.min(p3, axis=0))
    ep = jnp.exp2(p3 - mx[None])
    en = jnp.exp2(mn[None] - p3)
    sp = _fold4(jnp.add, jnp.sum(ep, axis=0))
    sn = _fold4(jnp.add, jnp.sum(en, axis=0))
    return ep, en, sp, sn


def _iota(shape, dim):
    return jax.lax.broadcasted_iota(jnp.int32, shape, dim)


def _kernel(x_hbm, wqkv_hbm, wphi_hbm, wo_hbm, w1_hbm, w2_hbm, w3t_hbm, w4_hbm, gate_ref,
            o_hbm,
            xs, wq_s, wk_s, wv_s, wphi_s, wo_s, w1_s, w2_s, w3t_s, w4_s, os_,
            wT, hbuf, kvacc, zacc, kvT, zb, wsem, xsem, osem):
    cp_phi = pltpu.make_async_copy(wphi_hbm, wphi_s, wsem.at[0])
    cp_wk = pltpu.make_async_copy(wqkv_hbm.at[:, D:2 * D], wk_s, wsem.at[1])
    cp_wv = pltpu.make_async_copy(wqkv_hbm.at[:, 2 * D:3 * D], wv_s, wsem.at[2])
    cp_w1 = pltpu.make_async_copy(w1_hbm, w1_s, wsem.at[3])
    cp_wq = pltpu.make_async_copy(wqkv_hbm.at[:, 0:D], wq_s, wsem.at[4])
    cp_w2 = pltpu.make_async_copy(w2_hbm, w2_s, wsem.at[5])
    cp_w3 = pltpu.make_async_copy(w3t_hbm, w3t_s, wsem.at[6])
    cp_w4 = pltpu.make_async_copy(w4_hbm, w4_s, wsem.at[7])
    cp_wo = pltpu.make_async_copy(wo_hbm, wo_s, wsem.at[8])

    def cp_x(i):
        return pltpu.make_async_copy(x_hbm.at[pl.ds(i * TM1, TM1), :],
                                     xs.at[pl.ds(i * TM1, TM1), :], xsem.at[i])

    def cp_o(i):
        return pltpu.make_async_copy(os_.at[pl.ds(i * TM2, TM2), :],
                                     o_hbm.at[pl.ds(i * TM2, TM2), :], osem.at[i])

    cp_phi.start()
    cp_wk.start()
    cp_wv.start()
    cp_x(0).start()
    cp_w1.start()
    for i in range(1, NB1):
        cp_x(i).start()
    cp_wq.start()
    cp_w2.start()
    cp_w3.start()
    cp_w4.start()
    cp_wo.start()

    kvacc[...] = jnp.zeros_like(kvacc)
    zacc[...] = jnp.zeros_like(zacc)
    for g in range(4):
        hbuf[g, 0:8, :] = jnp.zeros((8, 128), F32)
        hbuf[g, S + 8:S + 16, :] = jnp.zeros((8, 128), F32)

    cp_phi.wait()
    sel = jnp.where(_iota((H, D), 0) == _iota((H, D), 1) // DH, 1.0, 0.0).astype(BF)
    t = jnp.dot(wphi_s[...], sel, preferred_element_type=F32)
    t = jnp.where(_iota((256, D), 0) // DH == _iota((256, D), 1) % DH, t, 0.0).astype(BF)
    asel = jnp.where((_iota((128, 256), 0) % 64) // 4 == _iota((128, 256), 1) % DH,
                     1.0, 0.0).astype(BF)
    bdt = jnp.dot(asel, t, preferred_element_type=F32)
    rr = _iota((128, D), 0)
    hl8 = (rr // 64) * 4 + rr % 4
    bdt = jnp.where(hl8 == (_iota((128, D), 1) % 128) // DH, bdt, 0.0).astype(BF)
    eye = jnp.where(_iota((128, 128), 0) == _iota((128, 128), 1), 1.0, 0.0).astype(BF)

    def fold(w_s, row0):
        for j in range(4):
            wt = jax.lax.dot_general(bdt[:, j * 128:(j + 1) * 128],
                                     w_s[:, j * 128:(j + 1) * 128], NT,
                                     preferred_element_type=F32)
            wT[row0 + j * 128: row0 + (j + 1) * 128, :] = (wt * LOG2E).astype(BF)

    cp_wk.wait()
    fold(wk_s, D)
    cp_wv.wait()
    for j in range(4):
        wt = jax.lax.dot_general(eye, wv_s[:, j * 128:(j + 1) * 128], NT,
                                 preferred_element_type=F32)
        wT[2 * D + j * 128: 2 * D + (j + 1) * 128, :] = wt.astype(BF)
    cp_w1.wait()

    def p1(i, _):
        cp_x(i).wait()
        s0 = pl.multiple_of(i * TM1, TM1)
        xb = xs[pl.ds(s0, TM1), :]
        pkT = jax.lax.dot_general(wT[D:2 * D, :], xb, NT, preferred_element_type=F32)
        xn = _ln(xb.astype(F32)).astype(BF)
        h = _gelu(jnp.dot(xn, w1_s[...], preferred_element_type=F32))
        for g in range(4):
            hbuf[g, pl.ds(s0 + 8, TM1), :] = h[:, g * 128:(g + 1) * 128]
        vT = jax.lax.dot_general(wT[2 * D:3 * D, :], xb, NT,
                                 preferred_element_type=F32).astype(BF)
        for g in range(G):
            ep, en, sp, sn = _dual_exp(pkT[g * 64:(g + 1) * 64, :])
            pp = (ep * (1.0 / sp)[None]).reshape(64, TM1)
            pn = (en * (1.0 / sn)[None]).reshape(64, TM1)
            phi = jnp.concatenate([pp, pn], axis=0)
            zpart = phi[:, 0:128]
            for l in range(1, TM1 // 128):
                zpart = zpart + phi[:, l * 128:(l + 1) * 128]
            zacc[g] += zpart
            kvacc[g] += jax.lax.dot_general(vT[g * 64:(g + 1) * 64, :], phi.astype(BF), NT,
                                            preferred_element_type=F32)
        return 0

    jax.lax.fori_loop(0, NB1, p1, 0)

    cp_wq.wait()
    fold(wq_s, 0)
    m2 = _iota((64, 128), 0) // DH == _iota((64, 128), 1) % 4
    for g in range(G):
        kvT[g] = jnp.where(m2, kvacc[g], 0.0).astype(BF)
        zb[g] = jnp.broadcast_to(jnp.sum(zacc[g], axis=-1, keepdims=True), (128, 128))
    cp_w2.wait()
    cp_w3.wait()
    cp_w4.wait()
    cp_wo.wait()

    def p2(i, _):
        s0 = pl.multiple_of(i * TM2, TM2)
        xb = xs[pl.ds(s0, TM2), :]
        xf = xb.astype(F32)
        hsh = jnp.concatenate([
            hbuf[0, pl.ds(s0 + 7, TM2), :],
            hbuf[1, pl.ds(s0 + 9, TM2), :],
            hbuf[2, pl.ds(s0 + 6, TM2), :],
            hbuf[3, pl.ds(s0 + 10, TM2), :]], axis=1).astype(BF)
        x1 = xf + jnp.dot(hsh, w2_s[...], preferred_element_type=F32)
        pqT = jax.lax.dot_general(wT[0:D, :], xb, NT, preferred_element_type=F32)
        xn = _ln(x1).astype(BF)
        y = _gelu(jax.lax.dot_general(xn, w3t_s[...], NT,
                                      preferred_element_type=F32)).astype(BF)
        oT = []
        for g in range(G):
            ep, en, sp, sn = _dual_exp(pqT[g * 64:(g + 1) * 64, :])
            z = zb[g]
            zt = jnp.concatenate([z] * (TM2 // 128), axis=1).reshape(2, 8, 8, TM2)
            rp = 1.0 / sp
            rn = 1.0 / sn
            den = _fold4(jnp.add, jnp.sum(ep * zt[0], axis=0) * rp
                         + jnp.sum(en * zt[1], axis=0) * rn)
            inv = 1.0 / (den + 1e-6)
            pp = (ep * (rp * inv)[None]).reshape(64, TM2)
            pn = (en * (rn * inv)[None]).reshape(64, TM2)
            phi = jnp.concatenate([pp, pn], axis=0).astype(BF)
            oT.append(jnp.dot(kvT[g], phi, preferred_element_type=F32))
        o = jnp.concatenate(oT, axis=0).T.astype(BF)
        b = x1 + jnp.dot(y, w4_s[...], preferred_element_type=F32)
        a = jnp.dot(o, wo_s[...], preferred_element_type=F32)
        gl = jnp.sum(xf * gate_ref[...].astype(F32).reshape(1, D), axis=-1, keepdims=True)
        g = jax.nn.sigmoid(gl)
        os_[pl.ds(s0, TM2), :] = (b + g * (a - b)).astype(BF)
        cp_o(i).start()
        return 0

    jax.lax.fori_loop(0, NB2, p2, 0)
    for i in range(NB2):
        cp_o(i).wait()


@jax.jit
def pallas_gated_mix__linear_kernel_hedgehog__mixer_s_mlp__prompt_kernel(
    A_x, A_wqkv, A_w_phi, A_wo, B_x, B_w1, B_w2, B_w3, B_w4, gate_w):
    x = A_x.reshape(S, D)
    wphi = jnp.transpose(A_w_phi, (1, 2, 0)).reshape(DH * DH, H)
    hbm = pl.BlockSpec(memory_space=pl.ANY)
    out = pl.pallas_call(
        _kernel,
        out_shape=jax.ShapeDtypeStruct((S, D), BF),
        in_specs=[hbm] * 8 + [pl.BlockSpec(memory_space=pltpu.VMEM)],
        out_specs=hbm,
        scratch_shapes=[
            pltpu.VMEM((S, D), BF),
            pltpu.VMEM((D, D), BF),
            pltpu.VMEM((D, D), BF),
            pltpu.VMEM((D, D), BF),
            pltpu.VMEM((DH * DH, H), BF),
            pltpu.VMEM((D, D), BF),
            pltpu.VMEM((D, D), BF),
            pltpu.VMEM((D, D), BF),
            pltpu.VMEM((F, D), BF),
            pltpu.VMEM((F, D), BF),
            pltpu.VMEM((S, D), BF),
            pltpu.VMEM((3 * D, D), BF),
            pltpu.VMEM((4, S + 16, 128), F32),
            pltpu.VMEM((G, 64, 128), F32),
            pltpu.VMEM((G, 128, 128), F32),
            pltpu.VMEM((G, 64, 128), BF),
            pltpu.VMEM((G, 128, 128), F32),
            pltpu.SemaphoreType.DMA((9,)),
            pltpu.SemaphoreType.DMA((NB1,)),
            pltpu.SemaphoreType.DMA((NB2,)),
        ],
        compiler_params=pltpu.CompilerParams(vmem_limit_bytes=100 * 2**20),
    )(x, A_wqkv, wphi, A_wo, B_w1, B_w2, B_w3.T, B_w4, gate_w)
    return out.reshape(1, S, D)
```

```python
import contextlib
import math
import os

import jax
import jax.numpy as jnp
import jax.experimental.pallas as pl
import jax.experimental.pallas.tpu as pltpu

S, D, H, DH, F = 2048, 512, 32, 16, 1376
E = os.environ.get
X0 = int(E('X0', 512))
SB1 = int(E('SB1', 256))
CH1 = int(E('CH1', 128))
TM2 = int(E('TM2', 1024))
CH2 = int(E('CH2', 128))
CH3 = int(E('CH3', 512))
SEG2 = E('SEG2', 'n0,p0,f0,p1,f1')
SEG3 = E('SEG3', 'h0,h1,h2,h3,v0,k0,v1,k1')
SEG4 = E('SEG4', '')
DROP = int(E('DROP', 1))
FT = int(E('FT', 1))
LNMODE = int(E('LNMODE', 0))
SM = int(E('SM', 0))
NW = int(E('NW', 128))
PHIS = int(E('PHIS', 0))
PHIQ = int(E('PHIQ', 0))
ZREF = int(E('ZREF', 0))
SB2 = int(E('SB2', 1024))
ORDER2 = E('ORDER2', 'w0,q0,t0,n0,o0')
OCH = E('OCH', '256+256')
LASTCH = E('LASTCH', '512+384+64+64')
DMAO = int(E('DMAO', 0))
GEARLY = int(E('GEARLY', 0))
SCOPES = int(E('SCOPES', 0))
PR = 480 if DROP else 512
FM = 1280
NB2 = S // TM2
LOG2E = math.log2(math.e)
GELU_C = math.sqrt(2.0 / math.pi)
BF = jnp.bfloat16
F32 = jnp.float32
NT = (((1,), (1,)), ((), ()))
G = 8


def _scope(name):
    return jax.named_scope(name) if SCOPES else contextlib.nullcontext()


def _gelu(y, half=0.5):
    inner = y * (GELU_C + (GELU_C * 0.044715) * (y * y))
    hy = half * y
    return hy + hy * jnp.tanh(inner)


def _ln(xf):
    m = jnp.mean(xf, axis=-1, keepdims=True)
    if LNMODE == 2:
        v = jnp.maximum(jnp.mean(xf * xf, axis=-1, keepdims=True) - m * m, 0.0)
        return (xf - m) * jax.lax.rsqrt(v + 1e-5)
    xc = xf - m
    v = jnp.mean(xc * xc, axis=-1, keepdims=True)
    r = jax.lax.rsqrt(v + 1e-5)
    if LNMODE == 1:
        return xf * r - m * r
    return xc * r


def _tile(x, n):
    return jnp.concatenate([x] * n, axis=1)


def _rcp(x):
    return pl.reciprocal(x, approx=True)


def _fold4(op, t):
    return op(t, pltpu.roll(t, 4, 0))


def _group_rows(pT, g):
    T = pT.shape[-1]
    if not DROP:
        return pT[g * 64:(g + 1) * 64, :].reshape(8, 8, T)
    j, gl = g // 2, g % 2
    base = j * 120
    x = pT[base: base + 8, :]
    body = pT[base + 8 + gl * 56: base + 8 + (gl + 1) * 56, :]
    lo = _iota((8, T), 0) < 4
    last = jnp.where(lo, x, 0.0) if gl == 0 else jnp.where(lo, 0.0, x)
    return jnp.concatenate([last, body], axis=0).reshape(8, 8, T)


def _dual_exp(p3):
    mx = _fold4(jnp.maximum, jnp.max(p3, axis=0))
    mn = _fold4(jnp.minimum, jnp.min(p3, axis=0))
    ep = jnp.exp2(p3 - mx[None])
    en = jnp.exp2(mn[None] - p3)
    sp = _fold4(jnp.add, jnp.sum(ep, axis=0))
    sn = _fold4(jnp.add, jnp.sum(en, axis=0))
    return ep, en, sp, sn, mx, mn


def _iota(shape, dim):
    return jax.lax.broadcasted_iota(jnp.int32, shape, dim)


def _kernel(x_hbm, wqkv_hbm, wphi_hbm, wo_hbm, w1_hbm, w2_hbm, w3t_hbm, w4_hbm, gate_hbm,
            o_hbm,
            xs, wq_s, wk_s, wv_s, wphi_s, wo_s, w1_s, w2_s, w3t_s, w4_s, gate_s, os_,
            wT, hbuf, kvT, zb, phik, phiq, zref, sem):
    cp = pltpu.make_async_copy
    cp_phi = cp(wphi_hbm, wphi_s, sem.at[0])
    cp_wk = cp(wqkv_hbm.at[:, D:2 * D], wk_s, sem.at[1])
    cp_x0 = cp(x_hbm.at[0:X0, :], xs.at[0:X0, :], sem.at[2])
    cp_w1 = cp(w1_hbm, w1_s, sem.at[3])
    cp_wv = cp(wqkv_hbm.at[:, 2 * D:3 * D], wv_s, sem.at[3])
    cp_xr = cp(x_hbm.at[X0:S, :], xs.at[X0:S, :], sem.at[0])
    cp_wq = cp(wqkv_hbm.at[:, 0:D], wq_s, sem.at[0])
    late = [cp(w2_hbm, w2_s, sem.at[1]),
            cp(w3t_hbm, w3t_s, sem.at[1]),
            cp(w4_hbm, w4_s, sem.at[1]),
            cp(wo_hbm, wo_s, sem.at[1]),
            cp(gate_hbm, gate_s, sem.at[1])]

    cp_phi.start()
    cp_wk.start()

    def put_wT(r0, val):
        n = val.shape[0]
        wT[r0 // 2:(r0 + n) // 2, :] = pltpu.bitcast(val, jnp.uint32)

    def get_wT(r0, n):
        return pltpu.bitcast(wT[r0 // 2:(r0 + n) // 2, :], BF)

    def proj(r0, n, xb):
        T = xb.shape[0]
        return jnp.concatenate(
            [jax.lax.dot_general(get_wT(r0, n), xb[l:l + NW], NT, preferred_element_type=F32)
             for l in range(0, T, NW)], axis=1)

    with _scope('bdt'):
        for g in range(4):
            hbuf[g, 0:8, :] = jnp.zeros((8, 128), F32)
            hbuf[g, S + 8:S + 16, :] = jnp.zeros((8, 128), F32)

        cp_phi.wait()
        cp_x0.start()
        if not DMAO:
            cp_w1.start()
            cp_wv.start()
        sel = jnp.where(_iota((H, D), 0) == _iota((H, D), 1) // DH, 1.0, 0.0).astype(BF)
        t = jnp.dot(wphi_s[...], sel, preferred_element_type=F32)
        t = jnp.where(_iota((256, D), 0) // DH == _iota((256, D), 1) % DH, t, 0.0).astype(BF)
        asel = jnp.where((_iota((128, 256), 0) % 64) // 4 == _iota((128, 256), 1) % DH,
                         1.0, 0.0).astype(BF)
        bdt = jnp.dot(asel, t, preferred_element_type=F32)
        rr = _iota((128, D), 0)
        hl8 = (rr // 64) * 4 + rr % 4
        bdt = jnp.where(hl8 == (_iota((128, D), 1) % 128) // DH, bdt, 0.0).astype(BF)

    def fold(w_s, row0):
        pend = []
        for j in range(4):
            wt = jax.lax.dot_general(bdt[:, j * 128:(j + 1) * 128],
                                     w_s[:, j * 128:(j + 1) * 128], NT,
                                     preferred_element_type=F32)
            wt = wt * LOG2E
            if not DROP:
                put_wT(row0 + j * 128, wt.astype(BF))
                continue
            w4d = wt.reshape(2, 8, 8, D)
            lo = _iota((8, D), 0) < 4
            parts, tails = [], []
            for gl in range(2):
                ref = w4d[gl, 7]
                f15 = jnp.where(lo, pltpu.roll(ref, 4, 0), ref)
                parts.append((w4d[gl, 0:7] - f15[None]).reshape(56, D))
                tails.append(ref - f15)
            pend += [tails[0] + pltpu.roll(tails[1], 4, 0)] + parts
            if j % 2 == 1:
                put_wT(row0 + (j - 1) * 120, jnp.concatenate(pend, axis=0).astype(BF))
                pend = []

    with _scope('foldk'):
        cp_wk.wait()
        if DMAO:
            cp_w1.start()
            cp_wv.start()
        fold(wk_s, D)

    st = {}
    kvacc = [None] * G
    zacc = [None] * G

    def do_pk(a):
        xb = xs[a * SB1:(a + 1) * SB1, :]
        st['pk', a] = proj(D, PR, xb)

    def do_v(a):
        xb = xs[a * SB1:(a + 1) * SB1, :]
        st['v', a] = proj(2 * D, D, xb)

    def do_ln(c):
        st['xn', c] = _ln(xs[c * CH1:(c + 1) * CH1, :].astype(F32)).astype(BF)

    def do_h(c):
        r0 = c * CH1
        if ('xn', c) not in st:
            do_ln(c)
        xn = st.pop(('xn', c))
        h = _gelu(jnp.dot(xn, w1_s[...], preferred_element_type=F32))
        for g in range(4):
            hbuf[g, r0 + 8:r0 + 8 + CH1, :] = h[:, g * 128:(g + 1) * 128]

    def do_phi(a):
        pkT = st.pop(('pk', a))
        phis = []
        for g in range(G):
            p3 = _group_rows(pkT, g)
            ep, en, sp, sn, mx, mn = _dual_exp(p3)
            if SM == 1:
                pp = jnp.exp2(p3 - (mx + jnp.log2(sp))[None]).reshape(64, SB1)
                pn = jnp.exp2((mn - jnp.log2(sn))[None] - p3).reshape(64, SB1)
            else:
                pp = (ep * _rcp(sp)[None]).reshape(64, SB1)
                pn = (en * _rcp(sn)[None]).reshape(64, SB1)
            phi = jnp.concatenate([pp, pn], axis=0)
            if ZREF == 2:
                for l in range(SB1 // 128):
                    zpart = phi[:, l * 128:(l + 1) * 128]
                    if zacc[g] is None:
                        zref[g] = zpart
                        zacc[g] = 1
                    else:
                        zref[g] += zpart
            else:
                zpart = phi[:, 0:128]
                for l in range(1, SB1 // 128):
                    zpart = zpart + phi[:, l * 128:(l + 1) * 128]
                if ZREF:
                    if zacc[g] is None:
                        zref[g] = zpart
                        zacc[g] = 1
                    else:
                        zref[g] += zpart
                else:
                    zacc[g] = zpart if zacc[g] is None else zacc[g] + zpart
            if PHIS:
                phik[g * 64:(g + 1) * 64, a * SB1:(a + 1) * SB1] = pltpu.bitcast(
                    phi.astype(BF), jnp.uint32)
                phis.append(None)
            else:
                phis.append(phi.astype(BF))
        st['phi', a] = phis

    def do_kv(a):
        if ('phi', a) not in st:
            do_phi(a)
        phis, vT = st.pop(('phi', a)), st.pop(('v', a))
        for g in range(G):
            if PHIS:
                phis[g] = pltpu.bitcast(phik[g * 64:(g + 1) * 64, a * SB1:(a + 1) * SB1], BF)
            kv = jax.lax.dot_general(vT[g * 64:(g + 1) * 64, :].astype(BF), phis[g], NT,
                                     preferred_element_type=F32)
            kvacc[g] = kv if kvacc[g] is None else kvacc[g] + kv

    def do_fq(_):
        fold(wq_s, 0)

    def do_fin(_):
        m2 = _iota((64, 128), 0) // DH == _iota((64, 128), 1) % 4
        for g in range(G):
            kvT[g] = jnp.where(m2, kvacc[g], 0.0).astype(BF)
            zb[g] = jnp.broadcast_to(jnp.sum(zref[g] if ZREF else zacc[g], axis=-1, keepdims=True), (128, 128))

    fns = dict(p=do_pk, v=do_v, h=do_h, k=do_kv, q=do_fq, z=do_fin, f=do_phi, n=do_ln)

    def run(order):
        for tok in order.split(','):
            fns[tok[0]](int(tok[1:]))

    n0 = X0 // SB1
    with _scope('seg2'):
        cp_x0.wait()
        cp_xr.start()
        cp_wq.start()
        run(SEG2)
    with _scope('seg3'):
        cp_w1.wait()
        cp_wv.wait()
        for c in late:
            c.start()
        put_wT(2 * D, wv_s[...].T)
        run(SEG3)
    with _scope('seg4'):
        cp_xr.wait()
        cp_wq.wait()
        if SEG4:
            order = SEG4
        else:
            toks = []
            nsb = S // SB1
            r = SB1 // CH1
            for a in range(n0, nsb):
                hs = ['h%d' % c for c in range(a * r, (a + 1) * r)]
                if a < nsb - 1:
                    toks += ['p%d' % a, 'v%d' % a] + hs + ['k%d' % a]
                else:
                    toks += ['p%d' % a, 'v%d' % a, 'q0', 'k%d' % a, 'z0'] + hs
            order = ','.join(toks)
        run(order)

    for c in late:
        c.wait()

    def p2(i, _):
        with _scope('p2body'):
            s0 = pl.multiple_of(i * TM2, TM2)
            gw = gate_s[...].astype(F32).reshape(1, D)
            s2 = {}

            def row(off):
                return pl.multiple_of(s0 + off, 64)

            def do_w(b):
                x1s, xns, ths = [], [], []
                for c in range(SB2 // CH2):
                    r0 = row(b * SB2 + c * CH2)
                    hsh = jnp.concatenate([
                        hbuf[0, pl.ds(r0 + 7, CH2), :],
                        hbuf[1, pl.ds(r0 + 9, CH2), :],
                        hbuf[2, pl.ds(r0 + 6, CH2), :],
                        hbuf[3, pl.ds(r0 + 10, CH2), :]], axis=1).astype(BF)
                    xf = xs[pl.ds(r0, CH2), :].astype(F32)
                    x1 = xf + jnp.dot(hsh, w2_s[...], preferred_element_type=F32)
                    if GEARLY:
                        ths.append(jnp.broadcast_to(
                            jnp.tanh(0.5 * jnp.sum(xf * gw, axis=-1, keepdims=True)), (CH2, 128)))
                    x1s.append(x1)
                    xns.append(_ln(x1))
                s2['x1', b] = jnp.concatenate(x1s, axis=0)
                s2['xn', b] = jnp.concatenate(xns, axis=0)
                if GEARLY:
                    s2['th', b] = jnp.concatenate(ths, axis=0)

            def do_q(b):
                s2['pq', b] = proj(0, PR, xs[pl.ds(row(b * SB2), SB2), :])

            def do_t(b):
                xn = s2.pop(('xn', b))
                ys = []
                for c in range(SB2 // CH3):
                    xc = xn[c * CH3:(c + 1) * CH3].astype(BF)
                    if GEARLY:
                        th = s2['th', b][c * CH3:(c + 1) * CH3]
                        ym = _gelu(jax.lax.dot_general(xc, w3t_s[0:FM, :], NT,
                                                       preferred_element_type=F32),
                                   _tile(0.25 - 0.25 * th, FM // 128))
                        yt = _gelu(jax.lax.dot_general(w3t_s[FM:F, :], xc, NT,
                                                       preferred_element_type=F32))
                        ys.append(jnp.concatenate([ym, yt.T * (0.5 - 0.5 * th)[:, :F - FM]], axis=1))
                        continue
                    ym = _gelu(jax.lax.dot_general(xc, w3t_s[0:FM, :], NT,
                                                   preferred_element_type=F32))
                    yt = _gelu(jax.lax.dot_general(w3t_s[FM:F, :], xc, NT,
                                                   preferred_element_type=F32))
                    ys.append(jnp.concatenate([ym, yt.T], axis=1))
                s2['y', b] = jnp.concatenate(ys, axis=0)

            def do_n(b):
                pqT = s2.pop(('pq', b))
                oT = []
                for g in range(G):
                    p3 = _group_rows(pqT, g)
                    ep, en, sp, sn, mx, mn = _dual_exp(p3)
                    z = zb[g]
                    zt = jnp.concatenate([z] * (SB2 // 128), axis=1).reshape(2, 8, 8, SB2)
                    rp = _rcp(sp)
                    rn = _rcp(sn)
                    den = _fold4(jnp.add, jnp.sum(ep * zt[0], axis=0) * rp
                                 + jnp.sum(en * zt[1], axis=0) * rn) + 1e-6
                    inv = _rcp(den)
                    pp = (ep * (rp * inv)[None]).reshape(64, SB2)
                    pn = (en * (rn * inv)[None]).reshape(64, SB2)
                    phi = jnp.concatenate([pp, pn], axis=0).astype(BF)
                    oT.append(jnp.dot(kvT[g], phi, preferred_element_type=F32))
                s2['o', b] = jnp.concatenate(oT, axis=0).T

            def do_o(b):
                x1, y, o = s2.pop(('x1', b)), s2.pop(('y', b)), s2.pop(('o', b))
                last = b == TM2 // SB2 - 1
                sizes = [int(v) for v in (LASTCH if last else OCH).split('+')]
                assert sum(sizes) == SB2
                off = 0
                for n in sizes:
                    r0 = row(b * SB2 + off)
                    rows = slice(off, off + n)
                    off += n
                    if GEARLY:
                        th = s2['th', b][rows]
                        res = (x1[rows] * _tile(0.5 - 0.5 * th, 4)
                               + jnp.dot(y[rows].astype(BF), w4_s[...],
                                         preferred_element_type=F32)
                               + jnp.dot((o[rows] * _tile(0.5 + 0.5 * th, 4)).astype(BF), wo_s[...],
                                         preferred_element_type=F32))
                        os_[pl.ds(r0, n), :] = res.astype(BF)
                        cp(os_.at[pl.ds(r0, n), :], o_hbm.at[pl.ds(r0, n), :],
                           sem.at[2]).start()
                        continue
                    bb = x1[rows] + jnp.dot(y[rows].astype(BF), w4_s[...],
                                            preferred_element_type=F32)
                    a = jnp.dot(o[rows].astype(BF), wo_s[...], preferred_element_type=F32)
                    gl = jnp.sum(xs[pl.ds(r0, n), :].astype(F32) * gw, axis=-1, keepdims=True)
                    g4 = 0.5 + 0.5 * jnp.tanh(0.5 * gl)
                    os_[pl.ds(r0, n), :] = (bb + g4 * (a - bb)).astype(BF)
                    cp(os_.at[pl.ds(r0, n), :], o_hbm.at[pl.ds(r0, n), :], sem.at[2]).start()

            f2 = dict(w=do_w, q=do_q, t=do_t, n=do_n, o=do_o)
            for tok in ORDER2.split(','):
                f2[tok[0]](int(tok[1:]))
        return 0

    with _scope('phase2'):
        jax.lax.fori_loop(0, NB2, p2, 0)
    with _scope('tail'):
        cp(os_, o_hbm, sem.at[2]).wait()


@jax.jit
def pallas_gated_mix__linear_kernel_hedgehog__mixer_s_mlp__prompt_kernel(
    A_x, A_wqkv, A_w_phi, A_wo, B_x, B_w1, B_w2, B_w3, B_w4, gate_w):
    x = A_x.reshape(S, D)
    wphi = jnp.transpose(A_w_phi, (1, 2, 0)).reshape(DH * DH, H)
    hbm = pl.BlockSpec(memory_space=pl.ANY)
    out = pl.pallas_call(
        _kernel,
        out_shape=jax.ShapeDtypeStruct((S, D), BF),
        in_specs=[hbm] * 9,
        out_specs=hbm,
        scratch_shapes=[
            pltpu.VMEM((S, D), BF),
            pltpu.VMEM((D, D), BF),
            pltpu.VMEM((D, D), BF),
            pltpu.VMEM((D, D), BF),
            pltpu.VMEM((DH * DH, H), BF),
            pltpu.VMEM((D, D), BF),
            pltpu.VMEM((D, D), BF),
            pltpu.VMEM((D, D), BF),
            pltpu.VMEM((F, D), BF),
            pltpu.VMEM((F, D), BF),
            pltpu.VMEM((D,), BF),
            pltpu.VMEM((S, D), BF),
            pltpu.VMEM((3 * D // 2, D), jnp.uint32),
            pltpu.VMEM((4, S + 16, 128), F32),
            pltpu.VMEM((G, 64, 128), BF),
            pltpu.VMEM((G, 128, 128), F32),
            pltpu.VMEM((G * 64, S), jnp.uint32),
            pltpu.VMEM((G * 64, TM2), jnp.uint32),
            pltpu.VMEM((G, 128, 128), F32),
            pltpu.SemaphoreType.DMA((4,)),
        ],
        compiler_params=pltpu.CompilerParams(vmem_limit_bytes=100 * 2**20),
    )(x, A_wqkv, wphi, A_wo, B_w1, B_w2, B_w3.T, B_w4, gate_w)
    return out.reshape(1, S, D)
```

```python
import math

import jax
import jax.numpy as jnp
import jax.experimental.pallas as pl
import jax.experimental.pallas.tpu as pltpu

S, D, H, DH, F = 2048, 512, 32, 16, 1376
G = 8
PR = 480
FM = 1280
SZ = (384, 256, 256, 256, 256, 256, 256, 128)
BND = tuple(sum(SZ[:i]) for i in range(len(SZ) + 1))
X0 = BND[2]
CH1 = 128
TM2 = 1024
CH2 = 64
CH3 = 512
OUT_CHUNKS = (512, 384, 96, 32)
LOG2E = math.log2(math.e)
GELU_C = math.sqrt(2.0 / math.pi)
BF = jnp.bfloat16
F32 = jnp.float32
NT = (((1,), (1,)), ((), ()))


def _iota(shape, dim):
    return jax.lax.broadcasted_iota(jnp.int32, shape, dim)


def _dot(a, b):
    return jnp.dot(a, b, preferred_element_type=F32)


def _dot_nt(a, b):
    return jax.lax.dot_general(a, b, NT, preferred_element_type=F32)


def _gelu(y):
    inner = y * (GELU_C + (GELU_C * 0.044715) * (y * y))
    hy = 0.5 * y
    return hy + hy * jnp.tanh(inner)


def _ln(xf):
    m = jnp.mean(xf, axis=-1, keepdims=True)
    xc = xf - m
    v = jnp.mean(xc * xc, axis=-1, keepdims=True)
    return xc * jax.lax.rsqrt(v + 1e-5)


def _rcp(x):
    return pl.reciprocal(x, approx=True)


def _fold4(op, t):
    return op(t, pltpu.roll(t, 4, 0))


def _group_rows(pT, g):
    T = pT.shape[-1]
    base = (g // 2) * 120
    gl = g % 2
    x = pT[base: base + 8, :]
    body = pT[base + 8 + gl * 56: base + 8 + (gl + 1) * 56, :]
    lo = _iota((8, T), 0) < 4
    first = jnp.where(lo, x, 0.0) if gl == 0 else jnp.where(lo, 0.0, x)
    return jnp.concatenate([first, body], axis=0).reshape(8, 8, T)


def _dual_exp(p3):
    mx = _fold4(jnp.maximum, jnp.max(p3, axis=0))
    mn = _fold4(jnp.minimum, jnp.min(p3, axis=0))
    ep = jnp.exp2(p3 - mx[None])
    en = jnp.exp2(mn[None] - p3)
    sp = _fold4(jnp.add, jnp.sum(ep, axis=0))
    sn = _fold4(jnp.add, jnp.sum(en, axis=0))
    return ep, en, sp, sn


def _kernel(x_hbm, wqkv_hbm, wphi_hbm, wo_hbm, w1_hbm, w2_hbm, w3t_hbm, w4_hbm, gate_hbm,
            o_hbm,
            xs, wq_s, wk_s, wv_s, wphi_s, wo_s, w1_s, w2_s, w3t_s, w4_s, gate_s, os_,
            wT, hbuf, kvT, zb, one_s, sem):
    cp = pltpu.make_async_copy
    HW = D // 2
    cp_phi = cp(wphi_hbm, wphi_s, sem.at[0])
    cp_wka = cp(wqkv_hbm.at[:, D:D + HW], wk_s.at[:, 0:HW], sem.at[1])
    cp_x0a = cp(x_hbm.at[0:BND[1], :], xs.at[0:BND[1], :], sem.at[2])
    grp_c = [cp(wqkv_hbm.at[:, D + HW:2 * D], wk_s.at[:, HW:D], sem.at[0]),
             cp(x_hbm.at[BND[1]:X0, :], xs.at[BND[1]:X0, :], sem.at[0])]
    grp_d = [cp(w1_hbm, w1_s, sem.at[1]),
             cp(wqkv_hbm.at[:, 2 * D:3 * D], wv_s, sem.at[1])]
    grp_e = [cp(x_hbm.at[X0:S, :], xs.at[X0:S, :], sem.at[2]),
             cp(wqkv_hbm.at[:, 0:D], wq_s, sem.at[2])]
    grp_f = [cp(w2_hbm, w2_s, sem.at[0]),
             cp(w3t_hbm, w3t_s, sem.at[0]),
             cp(w4_hbm, w4_s, sem.at[0]),
             cp(wo_hbm, wo_s, sem.at[0]),
             cp(gate_hbm, gate_s, sem.at[0])]
    out_sem = sem.at[1]

    def start(grp):
        for c in grp:
            c.start()

    def wait(grp):
        for c in grp:
            c.wait()

    start([cp_phi, cp_wka, cp_x0a])

    def put_wT(r0, val):
        wT[r0 // 2:(r0 + val.shape[0]) // 2, :] = pltpu.bitcast(val, jnp.uint32)

    def proj(r0, n, xb):
        return _dot_nt(pltpu.bitcast(wT[r0 // 2:(r0 + n) // 2, :], BF), xb)

    for g in range(4):
        hbuf[g, 0:8, :] = jnp.zeros((8, 128), F32)
        hbuf[g, S + 8:S + 16, :] = jnp.zeros((8, 128), F32)

    cp_phi.wait()
    start(grp_c)
    sel = jnp.where(_iota((H, D), 0) == _iota((H, D), 1) // DH, 1.0, 0.0).astype(BF)
    t = _dot(wphi_s[...], sel)
    t = jnp.where(_iota((256, D), 0) // DH == _iota((256, D), 1) % DH, t, 0.0).astype(BF)
    asel = jnp.where(_iota((64, 256), 0) // 4 == _iota((64, 256), 1) % DH, 1.0, 0.0).astype(BF)
    vrep = _dot(asel, t)
    hl = _iota((64, D), 0) % 4
    h8 = (_iota((64, D), 1) % 128) // DH
    bdt = jnp.concatenate([jnp.where(h8 == hl, vrep, 0.0),
                           jnp.where(h8 == hl + 4, vrep, 0.0)], axis=0).astype(BF)

    def fold(w_s, row0, js):
        pend = []
        for j in js:
            wt = _dot_nt(bdt[:, j * 128:(j + 1) * 128], w_s[:, j * 128:(j + 1) * 128]) * LOG2E
            w4d = wt.reshape(2, 8, 8, D)
            lo = _iota((8, D), 0) < 4
            parts, tails = [], []
            for gl in range(2):
                ref = w4d[gl, 7]
                f15 = jnp.where(lo, pltpu.roll(ref, 4, 0), ref)
                parts.append((w4d[gl, 0:7] - f15[None]).reshape(56, D))
                tails.append(ref - f15)
            pend += [tails[0] + pltpu.roll(tails[1], 4, 0)] + parts
            if j % 2 == 1:
                put_wT(row0 + (j - 1) * 120, jnp.concatenate(pend, axis=0).astype(BF))
                pend = []

    cp_wka.wait()
    start(grp_d)
    fold(wk_s, D, (0, 1))

    def main(_i, _c):
        pk, vt, xn1 = {}, {}, {}
        phis = {a: [None] * G for a in range(len(SZ))}
        kvacc = [None] * G
        zacc = [None] * G

        def xblk(a):
            return xs[BND[a]:BND[a + 1], :]

        def do_pk(a, half=None):
            if half is None:
                p = proj(D, PR, xblk(a))
                pk[a, 0], pk[a, 1] = p[:PR // 2], p[PR // 2:]
            else:
                pk[a, half] = proj(D + half * (PR // 2), PR // 2, xblk(a))

        def do_v(a):
            vt[a] = proj(2 * D, D, xblk(a))

        def do_ln(c):
            xn1[c] = _ln(xs[c * CH1:(c + 1) * CH1, :].astype(F32)).astype(BF)

        def do_h(c):
            if c not in xn1:
                do_ln(c)
            h = _gelu(_dot(xn1.pop(c), w1_s[...]))
            r0 = c * CH1 + 8
            for g in range(4):
                hbuf[g, r0:r0 + CH1, :] = h[:, g * 128:(g + 1) * 128]

        def do_hs(a):
            for c in range(BND[a] // CH1, BND[a + 1] // CH1):
                do_h(c)

        def do_phi(a, gs=range(G)):
            T = SZ[a]
            for g in gs:
                if phis[a][g] is not None:
                    continue
                ep, en, sp, sn = _dual_exp(_group_rows(pk[a, g // 4], g % 4))
                phi = jnp.concatenate([(ep * _rcp(sp)[None]).reshape(64, T),
                                       (en * _rcp(sn)[None]).reshape(64, T)], axis=0)
                zpart = phi[:, 0:128]
                for l in range(1, T // 128):
                    zpart = zpart + phi[:, l * 128:(l + 1) * 128]
                zacc[g] = zpart if zacc[g] is None else zacc[g] + zpart
                phis[a][g] = phi.astype(BF)

        def do_kv(a):
            do_phi(a)
            v = vt.pop(a)
            for g in range(G):
                kv = _dot_nt(v[g * 64:(g + 1) * 64, :].astype(BF), phis[a][g])
                kvacc[g] = kv if kvacc[g] is None else kvacc[g] + kv

        cp_x0a.wait()
        do_pk(0, 0)
        do_phi(0, range(4))

        wait(grp_c)
        start(grp_e)
        fold(wk_s, D, (2, 3))
        do_pk(1, 0)
        do_pk(0, 1)
        do_phi(1, range(4))
        do_phi(0, range(4, 8))
        do_pk(1, 1)
        do_ln(0)

        wait(grp_d)
        start(grp_f)
        put_wT(2 * D, wv_s[...].T)
        do_hs(0)
        do_hs(1)
        for a in range(2):
            do_v(a)
            do_kv(a)

        wait(grp_e)
        u, w = len(SZ) - 2, len(SZ) - 1
        for a in range(2, u):
            do_pk(a)
            do_v(a)
            do_hs(a)
            do_kv(a)
        do_pk(u)
        do_v(u)
        do_pk(w)
        do_kv(u)
        do_v(w)
        do_kv(w)
        same_head = _iota((64, 128), 0) // DH == _iota((64, 128), 1) % 4
        for g in range(G):
            kvT[g] = jnp.where(same_head, kvacc[g], 0.0).astype(BF)
            zb[g] = jnp.broadcast_to(jnp.sum(zacc[g], axis=-1, keepdims=True), (128, 128))
        fold(wq_s, 0, (0, 1, 2, 3))
        do_hs(u)
        do_hs(w)

        wait(grp_f)

        def p2(i, _):
            s0 = pl.multiple_of(i * TM2, TM2)
            gw = gate_s[...].astype(F32).reshape(1, D)

            x1s, xns = [], []
            for c in range(TM2 // CH2):
                r0 = pl.multiple_of(s0 + c * CH2, CH2)
                hsh = jnp.concatenate([
                    hbuf[0, pl.ds(r0 + 7, CH2), :],
                    hbuf[1, pl.ds(r0 + 9, CH2), :],
                    hbuf[2, pl.ds(r0 + 6, CH2), :],
                    hbuf[3, pl.ds(r0 + 10, CH2), :]],
                    axis=1).astype(BF)
                x1 = xs[pl.ds(r0, CH2), :].astype(F32) + _dot(hsh, w2_s[...])
                x1s.append(x1)
                xns.append(_ln(x1))
            x1 = jnp.concatenate(x1s, axis=0)
            xn = jnp.concatenate(xns, axis=0)

            pqT = proj(0, PR, xs[pl.ds(s0, TM2), :])

            ys = []
            for c in range(TM2 // CH3):
                xc = xn[c * CH3:(c + 1) * CH3].astype(BF)
                ym = _gelu(_dot_nt(xc, w3t_s[0:FM, :]))
                yt = _gelu(_dot_nt(w3t_s[FM:F, :], xc))
                ys.append(jnp.concatenate([ym, yt.T], axis=1))
            y = jnp.concatenate(ys, axis=0)

            oT = []
            for g in range(G):
                ep, en, sp, sn = _dual_exp(_group_rows(pqT, g))
                zt = jnp.concatenate([zb[g]] * (TM2 // 128), axis=1).reshape(2, 8, 8, TM2)
                rp = _rcp(sp)
                rn = _rcp(sn)
                den = _fold4(jnp.add, jnp.sum(ep * zt[0], axis=0) * rp
                             + jnp.sum(en * zt[1], axis=0) * rn) + 1e-6
                inv = _rcp(den)
                phi = jnp.concatenate([(ep * (rp * inv)[None]).reshape(64, TM2),
                                       (en * (rn * inv)[None]).reshape(64, TM2)], axis=0)
                oT.append(_dot(kvT[g], phi.astype(BF)))
            o = jnp.concatenate(oT, axis=0).T

            off = 0
            for n in OUT_CHUNKS:
                r0 = pl.multiple_of(s0 + off, 16)
                rows = slice(off, off + n)
                off += n
                b = x1[rows] + _dot(y[rows].astype(BF), w4_s[...])
                a = _dot(o[rows].astype(BF), wo_s[...])
                gl = jnp.sum(xs[pl.ds(r0, n), :].astype(F32) * gw, axis=-1, keepdims=True)
                gate = 0.5 + 0.5 * jnp.tanh(0.5 * gl)
                os_[pl.ds(r0, n), :] = (b + gate * (a - b)).astype(BF)
                cp(os_.at[pl.ds(r0, n), :], o_hbm.at[pl.ds(r0, n), :], out_sem).start()
            return 0

        jax.lax.fori_loop(0, S // TM2, p2, 0)
        return 0

    one_s[0] = 1
    jax.lax.fori_loop(0, one_s[0], main, 0)
    cp(os_, o_hbm, out_sem).wait()


def _compiler_params():
    base = dict(vmem_limit_bytes=100 * 2**20)
    try:
        return pltpu.CompilerParams(disable_bounds_checks=True,
                                    disable_semaphore_checks=True, **base)
    except TypeError:
        return pltpu.CompilerParams(**base)


@jax.jit
def pallas_gated_mix__linear_kernel_hedgehog__mixer_s_mlp__prompt_kernel(
    A_x: jax.Array,
    A_wqkv: jax.Array,
    A_w_phi: jax.Array,
    A_wo: jax.Array,
    B_x: jax.Array,
    B_w1: jax.Array,
    B_w2: jax.Array,
    B_w3: jax.Array,
    B_w4: jax.Array,
    gate_w: jax.Array,
):
    del B_x
    x = A_x.reshape(S, D)
    wphi = jnp.transpose(A_w_phi, (1, 2, 0)).reshape(DH * DH, H)
    hbm = pl.BlockSpec(memory_space=pl.ANY)
    out = pl.pallas_call(
        _kernel,
        out_shape=jax.ShapeDtypeStruct((S, D), BF),
        in_specs=[hbm] * 9,
        out_specs=hbm,
        scratch_shapes=[
            pltpu.VMEM((S, D), BF),
            pltpu.VMEM((D, D), BF),
            pltpu.VMEM((D, D), BF),
            pltpu.VMEM((D, D), BF),
            pltpu.VMEM((DH * DH, H), BF),
            pltpu.VMEM((D, D), BF),
            pltpu.VMEM((D, D), BF),
            pltpu.VMEM((D, D), BF),
            pltpu.VMEM((F, D), BF),
            pltpu.VMEM((F, D), BF),
            pltpu.VMEM((D,), BF),
            pltpu.VMEM((S, D), BF),
            pltpu.VMEM((3 * D // 2, D), jnp.uint32),
            pltpu.VMEM((4, S + 16, 128), F32),
            pltpu.VMEM((G, 64, 128), BF),
            pltpu.VMEM((G, 128, 128), F32),
            pltpu.SMEM((1,), jnp.int32),
            pltpu.SemaphoreType.DMA((3,)),
        ],
        compiler_params=_compiler_params(),
    )(x, A_wqkv, wphi, A_wo, B_w1, B_w2, B_w3.T, B_w4, gate_w)
    return out.reshape(1, S, D)
```

```python
import math

import jax
import jax.numpy as jnp
import jax.experimental.pallas as pl
import jax.experimental.pallas.tpu as pltpu

S, D, H, DH, F = 2048, 512, 32, 16, 1376
G = 8
PR = 480
FM = 1280
SZ = (128, 128, 384, 128, 256, 256, 384, 256, 128)
BND = tuple(sum(SZ[:i]) for i in range(len(SZ) + 1))
NA, N0 = 2, 4
CH1 = 128
TM2 = 1024
CH2 = 64
CH3 = 512
OUT_CHUNKS = (512, 384, 96, 32)
LOG2E = math.log2(math.e)
GELU_C = math.sqrt(2.0 / math.pi)
BF = jnp.bfloat16
F32 = jnp.float32
NT = (((1,), (1,)), ((), ()))


def _iota(shape, dim):
    return jax.lax.broadcasted_iota(jnp.int32, shape, dim)


def _dot(a, b):
    return jnp.dot(a, b, preferred_element_type=F32)


def _dot_nt(a, b):
    return jax.lax.dot_general(a, b, NT, preferred_element_type=F32)


def _gelu(y):
    inner = y * (GELU_C + (GELU_C * 0.044715) * (y * y))
    hy = 0.5 * y
    return hy + hy * jnp.tanh(inner)


def _ln(xf):
    m = jnp.mean(xf, axis=-1, keepdims=True)
    xc = xf - m
    v = jnp.mean(xc * xc, axis=-1, keepdims=True)
    return xc * jax.lax.rsqrt(v + 1e-5)


def _rcp(x):
    return pl.reciprocal(x, approx=True)


def _fold4(op, t):
    return op(t, pltpu.roll(t, 4, 0))


def _group_rows(pT, g):
    T = pT.shape[-1]
    base = (g // 2) * 120
    gl = g % 2
    x = pT[base: base + 8, :]
    body = pT[base + 8 + gl * 56: base + 8 + (gl + 1) * 56, :]
    lo = _iota((8, T), 0) < 4
    first = jnp.where(lo, x, 0.0) if gl == 0 else jnp.where(lo, 0.0, x)
    return jnp.concatenate([first, body], axis=0).reshape(8, 8, T)


def _dual_exp(p3):
    mx = _fold4(jnp.maximum, jnp.max(p3, axis=0))
    mn = _fold4(jnp.minimum, jnp.min(p3, axis=0))
    ep = jnp.exp2(p3 - mx[None])
    en = jnp.exp2(mn[None] - p3)
    sp = _fold4(jnp.add, jnp.sum(ep, axis=0))
    sn = _fold4(jnp.add, jnp.sum(en, axis=0))
    return ep, en, sp, sn


def _kernel(x_hbm, wqkv_hbm, wphi_hbm, wo_hbm, w1_hbm, w2_hbm, w3t_hbm, w4_hbm, gate_hbm,
            o_hbm,
            xs, wq_s, wk_s, wv_s, wphi_s, wo_s, w1_s, w2_s, w3t_s, w4_s, gate_s, os_,
            wT, hbuf, kvT, zb, one_s, sem):
    cp = pltpu.make_async_copy
    HW = D // 2
    XA, X0 = BND[NA], BND[N0]
    cp_phi = cp(wphi_hbm, wphi_s, sem.at[0])
    cp_wka = cp(wqkv_hbm.at[:, D:D + HW], wk_s.at[:, 0:HW], sem.at[1])
    cp_wkb = cp(wqkv_hbm.at[:, D + HW:2 * D], wk_s.at[:, HW:D], sem.at[2])
    cp_xa = cp(x_hbm.at[0:XA, :], xs.at[0:XA, :], sem.at[3])
    cp_xb = cp(x_hbm.at[XA:X0, :], xs.at[XA:X0, :], sem.at[0])
    grp_d = [cp(w1_hbm, w1_s, sem.at[1]),
             cp(wqkv_hbm.at[:, 2 * D:3 * D], wv_s, sem.at[1])]
    grp_e = [cp(x_hbm.at[X0:S, :], xs.at[X0:S, :], sem.at[2]),
             cp(wqkv_hbm.at[:, 0:D], wq_s, sem.at[2])]
    grp_f = [cp(w2_hbm, w2_s, sem.at[3]),
             cp(w3t_hbm, w3t_s, sem.at[3]),
             cp(w4_hbm, w4_s, sem.at[3]),
             cp(wo_hbm, wo_s, sem.at[3]),
             cp(gate_hbm, gate_s, sem.at[3])]
    out_sem = sem.at[0]

    def start(grp):
        for c in grp:
            c.start()

    def wait(grp):
        for c in grp:
            c.wait()

    start([cp_phi, cp_wka, cp_wkb, cp_xa])

    def put_wT(r0, val):
        wT[r0 // 2:(r0 + val.shape[0]) // 2, :] = pltpu.bitcast(val, jnp.uint32)

    def proj(r0, n, xb):
        return _dot_nt(pltpu.bitcast(wT[r0 // 2:(r0 + n) // 2, :], BF), xb)

    for g in range(4):
        hbuf[g, 0:8, :] = jnp.zeros((8, 128), F32)
        hbuf[g, S + 8:S + 16, :] = jnp.zeros((8, 128), F32)

    cp_phi.wait()
    cp_xb.start()
    sel = jnp.where(_iota((H, D), 0) == _iota((H, D), 1) // DH, 1.0, 0.0).astype(BF)
    t = _dot(wphi_s[...], sel)
    t = jnp.where(_iota((256, D), 0) // DH == _iota((256, D), 1) % DH, t, 0.0).astype(BF)
    asel = jnp.where(_iota((64, 256), 0) // 4 == _iota((64, 256), 1) % DH, 1.0, 0.0).astype(BF)
    vrep = _dot(asel, t)
    hl = _iota((64, D), 0) % 4
    h8 = (_iota((64, D), 1) % 128) // DH
    bdt = jnp.concatenate([jnp.where(h8 == hl, vrep, 0.0),
                           jnp.where(h8 == hl + 4, vrep, 0.0)], axis=0).astype(BF)

    def fold(w_s, row0, js):
        pend = []
        for j in js:
            wt = _dot_nt(bdt[:, j * 128:(j + 1) * 128], w_s[:, j * 128:(j + 1) * 128]) * LOG2E
            w4d = wt.reshape(2, 8, 8, D)
            lo = _iota((8, D), 0) < 4
            parts, tails = [], []
            for gl in range(2):
                ref = w4d[gl, 7]
                f15 = jnp.where(lo, pltpu.roll(ref, 4, 0), ref)
                parts.append((w4d[gl, 0:7] - f15[None]).reshape(56, D))
                tails.append(ref - f15)
            pend += [tails[0] + pltpu.roll(tails[1], 4, 0)] + parts
            if j % 2 == 1:
                put_wT(row0 + (j - 1) * 120, jnp.concatenate(pend, axis=0).astype(BF))
                pend = []

    cp_wka.wait()
    start(grp_d)
    fold(wk_s, D, (0, 1))
    cp_wkb.wait()
    fold(wk_s, D, (2, 3))

    def main(_i, _c):
        pk, vt, xn1 = {}, {}, {}
        phis = {}
        kvacc = [None] * G
        zacc = [None] * G

        def xblk(a):
            return xs[BND[a]:BND[a + 1], :]

        def do_pk(a):
            pk[a] = proj(D, PR, xblk(a))

        def do_v(a):
            vt[a] = proj(2 * D, D, xblk(a))

        def do_ln(c):
            xn1[c] = _ln(xs[c * CH1:(c + 1) * CH1, :].astype(F32)).astype(BF)

        def do_h(c):
            if c not in xn1:
                do_ln(c)
            h = _gelu(_dot(xn1.pop(c), w1_s[...]))
            r0 = c * CH1 + 8
            for g in range(4):
                hbuf[g, r0:r0 + CH1, :] = h[:, g * 128:(g + 1) * 128]

        def do_hs(a):
            for c in range(BND[a] // CH1, BND[a + 1] // CH1):
                do_h(c)

        def do_phi(a):
            if a in phis:
                return
            T = SZ[a]
            phis[a] = []
            p = pk.pop(a)
            for g in range(G):
                ep, en, sp, sn = _dual_exp(_group_rows(p, g))
                phi = jnp.concatenate([(ep * _rcp(sp)[None]).reshape(64, T),
                                       (en * _rcp(sn)[None]).reshape(64, T)], axis=0)
                zpart = phi[:, T - 128:]
                for l in range(T // 128 - 2, -1, -1):
                    zpart = zpart + phi[:, l * 128:(l + 1) * 128]
                zacc[g] = zpart if zacc[g] is None else zpart + zacc[g]
                phis[a].append(phi.astype(BF))

        def do_kv(a):
            do_phi(a)
            v = vt.pop(a)
            for g in range(G):
                kv = _dot_nt(v[g * 64:(g + 1) * 64, :].astype(BF), phis[a][g])
                kvacc[g] = kv if kvacc[g] is None else kvacc[g] + kv

        cp_xa.wait()
        for a in range(NA):
            do_pk(a)
            if a < NA - 1:
                do_phi(a)

        cp_xb.wait()
        start(grp_e)
        for a in range(NA, N0):
            do_pk(a)
            if a < N0 - 1:
                do_phi(a)
        do_ln(0)

        wait(grp_d)
        start(grp_f)
        put_wT(2 * D, wv_s[...].T)
        for a in range(N0):
            do_hs(a)
        for a in range(N0):
            do_v(a)
            do_kv(a)

        wait(grp_e)
        u, w = len(SZ) - 2, len(SZ) - 1
        for a in range(N0, u):
            do_pk(a)
            do_v(a)
            do_hs(a)
            do_kv(a)
        do_pk(u)
        do_v(u)
        do_pk(w)
        do_kv(u)
        do_v(w)
        do_kv(w)
        same_head = _iota((64, 128), 0) // DH == _iota((64, 128), 1) % 4
        for g in range(G):
            kvT[g] = jnp.where(same_head, kvacc[g], 0.0).astype(BF)
            zb[g] = jnp.broadcast_to(jnp.sum(zacc[g], axis=-1, keepdims=True), (128, 128))
        fold(wq_s, 0, (0, 1, 2, 3))
        do_hs(u)
        do_hs(w)

        wait(grp_f)

        def p2(i, _):
            s0 = pl.multiple_of(i * TM2, TM2)
            gw = gate_s[...].astype(F32).reshape(1, D)

            x1s, xns = [], []
            for c in range(TM2 // CH2):
                r0 = pl.multiple_of(s0 + c * CH2, CH2)
                hsh = jnp.concatenate([
                    hbuf[0, pl.ds(r0 + 7, CH2), :],
                    hbuf[1, pl.ds(r0 + 9, CH2), :],
                    hbuf[2, pl.ds(r0 + 6, CH2), :],
                    hbuf[3, pl.ds(r0 + 10, CH2), :]],
                    axis=1).astype(BF)
                x1 = xs[pl.ds(r0, CH2), :].astype(F32) + _dot(hsh, w2_s[...])
                x1s.append(x1)
                xns.append(_ln(x1))
            x1 = jnp.concatenate(x1s, axis=0)
            xn = jnp.concatenate(xns, axis=0)

            ys = []
            for c in range(TM2 // CH3):
                if c == 1:
                    pqT = proj(0, PR, xs[pl.ds(s0, TM2), :])
                xc = xn[c * CH3:(c + 1) * CH3].astype(BF)
                ym = _gelu(_dot_nt(xc, w3t_s[0:FM, :]))
                yt = _gelu(_dot_nt(w3t_s[FM:F, :], xc))
                ys.append(jnp.concatenate([ym, yt.T], axis=1))
            y = jnp.concatenate(ys, axis=0)

            oT = []
            for g in range(G):
                ep, en, sp, sn = _dual_exp(_group_rows(pqT, g))
                zt = jnp.concatenate([zb[g]] * (TM2 // 128), axis=1).reshape(2, 8, 8, TM2)
                rp = _rcp(sp)
                rn = _rcp(sn)
                den = _fold4(jnp.add, jnp.sum(ep * zt[0], axis=0) * rp
                             + jnp.sum(en * zt[1], axis=0) * rn) + 1e-6
                inv = _rcp(den)
                phi = jnp.concatenate([(ep * (rp * inv)[None]).reshape(64, TM2),
                                       (en * (rn * inv)[None]).reshape(64, TM2)], axis=0)
                oT.append(_dot(kvT[g], phi.astype(BF)))
            o = jnp.concatenate(oT, axis=0).T

            off = 0
            for n in OUT_CHUNKS:
                r0 = pl.multiple_of(s0 + off, 16)
                rows = slice(off, off + n)
                off += n
                b = x1[rows] + _dot(y[rows].astype(BF), w4_s[...])
                a = _dot(o[rows].astype(BF), wo_s[...])
                gl = jnp.sum(xs[pl.ds(r0, n), :].astype(F32) * gw, axis=-1, keepdims=True)
                gate = 0.5 + 0.5 * jnp.tanh(0.5 * gl)
                os_[pl.ds(r0, n), :] = (b + gate * (a - b)).astype(BF)
                cp(os_.at[pl.ds(r0, n), :], o_hbm.at[pl.ds(r0, n), :], out_sem).start()
            return 0

        jax.lax.fori_loop(0, S // TM2, p2, 0)
        return 0

    one_s[0] = 1
    jax.lax.fori_loop(0, one_s[0], main, 0)
    cp(os_, o_hbm, out_sem).wait()


def _compiler_params():
    base = dict(vmem_limit_bytes=100 * 2**20)
    try:
        return pltpu.CompilerParams(disable_bounds_checks=True,
                                    disable_semaphore_checks=True, **base)
    except TypeError:
        return pltpu.CompilerParams(**base)


@jax.jit
def pallas_gated_mix__linear_kernel_hedgehog__mixer_s_mlp__prompt_kernel(
    A_x: jax.Array,
    A_wqkv: jax.Array,
    A_w_phi: jax.Array,
    A_wo: jax.Array,
    B_x: jax.Array,
    B_w1: jax.Array,
    B_w2: jax.Array,
    B_w3: jax.Array,
    B_w4: jax.Array,
    gate_w: jax.Array,
):
    del B_x
    x = A_x.reshape(S, D)
    wphi = jnp.transpose(A_w_phi, (1, 2, 0)).reshape(DH * DH, H)
    hbm = pl.BlockSpec(memory_space=pl.ANY)
    out = pl.pallas_call(
        _kernel,
        out_shape=jax.ShapeDtypeStruct((S, D), BF),
        in_specs=[hbm] * 9,
        out_specs=hbm,
        scratch_shapes=[
            pltpu.VMEM((S, D), BF),
            pltpu.VMEM((D, D), BF),
            pltpu.VMEM((D, D), BF),
            pltpu.VMEM((D, D), BF),
            pltpu.VMEM((DH * DH, H), BF),
            pltpu.VMEM((D, D), BF),
            pltpu.VMEM((D, D), BF),
            pltpu.VMEM((D, D), BF),
            pltpu.VMEM((F, D), BF),
            pltpu.VMEM((F, D), BF),
            pltpu.VMEM((D,), BF),
            pltpu.VMEM((S, D), BF),
            pltpu.VMEM((3 * D // 2, D), jnp.uint32),
            pltpu.VMEM((4, S + 16, 128), F32),
            pltpu.VMEM((G, 64, 128), BF),
            pltpu.VMEM((G, 128, 128), F32),
            pltpu.SMEM((1,), jnp.int32),
            pltpu.SemaphoreType.DMA((4,)),
        ],
        compiler_params=_compiler_params(),
    )(x, A_wqkv, wphi, A_wo, B_w1, B_w2, B_w3.T, B_w4, gate_w)
    return out.reshape(1, S, D)
```

```python
import math
import os

import jax
import jax.numpy as jnp
import jax.experimental.pallas as pl
import jax.experimental.pallas.tpu as pltpu

S, D, H, DH, F = 2048, 512, 32, 16, 1376
G = 8
PR = 480
FM = 1280
SZ = (128, 128, 384, 128, 256, 256, 384, 256, 128)
BND = tuple(sum(SZ[:i]) for i in range(len(SZ) + 1))
NA, N0 = 2, 4
TM2 = 1024
OUT_CHUNKS = (512, 384, 96, 32)
E = os.environ.get
CH3 = int(E('CH3', 1024))
NJ = int(E('NJ', 128))
OC = [[int(v) for v in c.split('+')] for c in E('OC', '256+128+96+32').split(',')]
QPOS = int(E('QPOS', 0))
CASTLATE = int(E('CASTLATE', 1))
SWAP = int(E('SWAP', 1))
CH1 = int(E('CH1', 128))
CH2 = int(E('CH2', 128))
SW1 = int(E('SW1', 0))
SW2 = int(E('SW2', 1))
SWO = int(E('SWO', 1))
G5 = int(E('G5', 1))
RS = int(E('RS', 0))
NW1 = int(E('NW1', 256))
NW2 = int(E('NW2', 256))
NWO = int(E('NWO', 256))
NW4 = int(E('NW4', 256))
PRE = int(E('PRE', 0))
PSTEP = int(E('PSTEP', 16))
SEG4 = E('SEG4', 'c0,p4,v4,h4,k4,p5,v5,h5,k5,c1,p6,v6,h6,k6,p7,v7,p8,k7,v8,k8,z0,q0,h7,h8')
TAILF = int(E('TAILF', 1))
WORDS = int(E('WORDS', 0))
LNM = int(E('LNM', 0))
YB = int(E('YB', 0))
ORD3 = [int(v) for v in E('ORD3', '4213065')]
ORD4 = [int(v) for v in E('ORD4', '4213065')]
LOG2E = math.log2(math.e)
GELU_C = math.sqrt(2.0 / math.pi)
BF = jnp.bfloat16
F32 = jnp.float32
NT = (((1,), (1,)), ((), ()))


def _iota(shape, dim):
    return jax.lax.broadcasted_iota(jnp.int32, shape, dim)


def _dot(a, b):
    return jnp.dot(a, b, preferred_element_type=F32)


def _dot_nt(a, b):
    return jax.lax.dot_general(a, b, NT, preferred_element_type=F32)


def _lhs7(a11, a12, a21, a22):
    return [a11 + a22, a21 + a22, a11, a22, a11 + a12, a21 - a11, a12 - a22]


def _rhs7w(w11, w12, w21, w22):
    def halves(w):
        return (pltpu.bitcast(w << 16, F32), pltpu.bitcast(w & jnp.uint32(0xFFFF0000), F32))

    def pack(lo, hi):
        return pltpu.bitcast(pltpu.pack_elementwise([lo, hi], packed_dtype=BF), BF)

    f11, f12, f21, f22 = (halves(w) for w in (w11, w12, w21, w22))
    add = lambda a, b: pack(a[0] + b[0], a[1] + b[1])
    sub = lambda a, b: pack(a[0] - b[0], a[1] - b[1])
    return [add(f11, f22), pltpu.bitcast(w11, BF), sub(f12, f22), sub(f21, f11),
            pltpu.bitcast(w22, BF), add(f11, f12), add(f21, f22)]


def _rhs7(b11, b12, b21, b22):
    f11, f12, f21, f22 = (b.astype(F32) for b in (b11, b12, b21, b22))
    return [(f11 + f22).astype(BF), b11, (f12 - f22).astype(BF), (f21 - f11).astype(BF),
            b22, (f11 + f12).astype(BF), (f21 + f22).astype(BF)]


_TERMS = (((0, 1), (3, 1), (4, -1), (6, 1)), ((2, 1), (4, 1)), ((1, 1), (3, 1)),
          ((0, 1), (1, -1), (2, 1), (5, 1)))


def _out4(m, order):
    outs = []
    for terms in _TERMS:
        terms = sorted(terms, key=lambda t: -order.index(t[0]))
        assert terms[0][1] == 1
        acc = m[terms[0][0]]
        for i, sg in terms[1:]:
            acc = acc + m[i] if sg > 0 else acc - m[i]
        outs.append(acc)
    return tuple(outs)


def _quads(a):
    h, k = a.shape[0] // 2, a.shape[1] // 2
    return a[:h, :k], a[:h, k:], a[h:, :k], a[h:, k:]


def _prep(ref, nw, r0=0, rows=None, swap=False):
    rows = rows or ref.shape[0]
    h, k = rows // 2, ref.shape[1] // 2
    t, u = (r0 + h, r0) if swap else (r0, r0 + h)
    if WORDS:
        w = ref.bitcast(jnp.uint32)
        t, u, h = t // 2, u // 2, h // 2
        return [_rhs7w(w[t:t + h, j:j + nw], w[t:t + h, k + j:k + j + nw],
                       w[u:u + h, j:j + nw], w[u:u + h, k + j:k + j + nw])
                for j in range(0, k, nw)]
    return [_rhs7(ref[t:t + h, j:j + nw], ref[t:t + h, k + j:k + j + nw],
                  ref[u:u + h, j:j + nw], ref[u:u + h, k + j:k + j + nw])
            for j in range(0, k, nw)]


def _prep_store(dst, ref, rows, swap=False, transposed=False, step=16):
    h, k = rows // 2, ref.shape[1] // 2
    t, u = (h, 0) if swap else (0, h)
    for r in range(0, h, step):
        q = [ref[t + r:t + r + step, 0:k], ref[t + r:t + r + step, k:2 * k],
             ref[u + r:u + r + step, 0:k], ref[u + r:u + r + step, k:2 * k]]
        if transposed:
            q = [q[0], q[2], q[1], q[3]]
        for i, v in enumerate(_rhs7(*q)):
            dst[i, r // 2:(r + step) // 2, :] = pltpu.bitcast(v, jnp.uint32)


def _prep_load(src, nw):
    k = src.shape[2]
    return [[pltpu.bitcast(src[i, :, j:j + nw], BF) for i in range(7)] for j in range(0, k, nw)]


def _smm7(l7, bt):
    outs = []
    for b7 in bt:
        m = [None] * 7
        for i in ORD4:
            m[i] = _dot(l7[i], b7[i])
        outs.append(_out4(m, ORD4))
    c11, c12, c21, c22 = ([o[q] for o in outs] for q in range(4))
    return jnp.concatenate(c11 + c12, axis=1), jnp.concatenate(c21 + c22, axis=1)


def _smm(quads, bt):
    return _smm7([v.astype(BF) for v in _lhs7(*quads)], bt)


GK = (GELU_C * 0.044715) ** (1.0 / 3.0)
GOUT = 0.5 / GK


def _gelu(y):
    if G5:
        return y + y * jnp.tanh(y * (GELU_C / GK + y * y))
    inner = y * (GELU_C + (GELU_C * 0.044715) * (y * y))
    hy = 0.5 * y
    return hy + hy * jnp.tanh(inner)


def _ln(xf):
    m = jnp.mean(xf, axis=-1, keepdims=True)
    if LNM == 2:
        v = jnp.maximum(jnp.mean(xf * xf, axis=-1, keepdims=True) - m * m, 0.0)
        xc = xf - m
    else:
        xc = xf - m
        v = jnp.mean(xc * xc, axis=-1, keepdims=True)
    if RS:
        r = jnp.exp2(-0.5 * jnp.log2(v + 1e-5) + (math.log2(GK) if G5 else 0.0))
    elif G5:
        r = jax.lax.rsqrt(v * (1.0 / GK ** 2) + 1e-5 / GK ** 2)
    else:
        r = jax.lax.rsqrt(v + 1e-5)
    return xc * r


def _rcp(x):
    return pl.reciprocal(x, approx=True)


def _fold4(op, t):
    return op(t, pltpu.roll(t, 4, 0))


def _group_rows(pT, g):
    T = pT.shape[-1]
    base = (g // 2) * 120
    gl = g % 2
    x = pT[base: base + 8, :]
    body = pT[base + 8 + gl * 56: base + 8 + (gl + 1) * 56, :]
    lo = _iota((8, T), 0) < 4
    first = jnp.where(lo, x, 0.0) if gl == 0 else jnp.where(lo, 0.0, x)
    return jnp.concatenate([first, body], axis=0).reshape(8, 8, T)


def _dual_exp(p3):
    mx = _fold4(jnp.maximum, jnp.max(p3, axis=0))
    mn = _fold4(jnp.minimum, jnp.min(p3, axis=0))
    ep = jnp.exp2(p3 - mx[None])
    en = jnp.exp2(mn[None] - p3)
    sp = _fold4(jnp.add, jnp.sum(ep, axis=0))
    sn = _fold4(jnp.add, jnp.sum(en, axis=0))
    return ep, en, sp, sn


def _kernel(x_hbm, wqkv_hbm, wphi_hbm, wo_hbm, w1_hbm, w2_hbm, w3t_hbm, w4_hbm, gate_hbm,
            o_hbm,
            xs, wq_s, wk_s, wv_s, wphi_s, wo_s, w1_s, w2_s, w3t_s, w4_s, gate_s, os_,
            wT, hbuf, kvT, zb, ybuf, c2, co, c3, c4, one_s, sem):
    cp = pltpu.make_async_copy
    HW = D // 2
    XA, X0 = BND[NA], BND[N0]
    cp_phi = cp(wphi_hbm, wphi_s, sem.at[0])
    cp_wka = cp(wqkv_hbm.at[:, D:D + HW], wk_s.at[:, 0:HW], sem.at[1])
    cp_wkb = cp(wqkv_hbm.at[:, D + HW:2 * D], wk_s.at[:, HW:D], sem.at[2])
    cp_xa = cp(x_hbm.at[0:XA, :], xs.at[0:XA, :], sem.at[3])
    cp_xb = cp(x_hbm.at[XA:X0, :], xs.at[XA:X0, :], sem.at[0])
    grp_d = [cp(w1_hbm, w1_s, sem.at[1]),
             cp(wqkv_hbm.at[:, 2 * D:3 * D], wv_s, sem.at[1])]
    grp_e = [cp(x_hbm.at[X0:S, :], xs.at[X0:S, :], sem.at[2]),
             cp(wqkv_hbm.at[:, 0:D], wq_s, sem.at[2]),
             cp(w2_hbm, w2_s, sem.at[2]),
             cp(wo_hbm, wo_s, sem.at[2])]
    grp_f = [cp(w3t_hbm, w3t_s, sem.at[3]),
             cp(w4_hbm, w4_s, sem.at[3]),
             cp(gate_hbm, gate_s, sem.at[3])]
    out_sem = sem.at[0]

    def start(grp):
        for c in grp:
            c.start()

    def wait(grp):
        for c in grp:
            c.wait()

    start([cp_phi, cp_wka, cp_wkb, cp_xa])

    def put_wT(r0, val):
        wT[r0 // 2:(r0 + val.shape[0]) // 2, :] = pltpu.bitcast(val, jnp.uint32)

    def proj(r0, n, xb):
        return _dot_nt(pltpu.bitcast(wT[r0 // 2:(r0 + n) // 2, :], BF), xb)

    for g in range(4):
        hbuf[g, 0:8, :] = jnp.zeros((8, 128), F32)
        hbuf[g, S + 8:S + 16, :] = jnp.zeros((8, 128), F32)

    cp_phi.wait()
    cp_xb.start()
    sel = jnp.where(_iota((H, D), 0) == _iota((H, D), 1) // DH, 1.0, 0.0).astype(BF)
    t = _dot(wphi_s[...], sel)
    t = jnp.where(_iota((256, D), 0) // DH == _iota((256, D), 1) % DH, t, 0.0).astype(BF)
    asel = jnp.where(_iota((64, 256), 0) // 4 == _iota((64, 256), 1) % DH, 1.0, 0.0).astype(BF)
    vrep = _dot(asel, t)
    hl = _iota((64, D), 0) % 4
    h8 = (_iota((64, D), 1) % 128) // DH
    bdt = jnp.concatenate([jnp.where(h8 == hl, vrep, 0.0),
                           jnp.where(h8 == hl + 4, vrep, 0.0)], axis=0).astype(BF)

    def fold(w_s, row0, js):
        pend = []
        for j in js:
            wt = _dot_nt(bdt[:, j * 128:(j + 1) * 128], w_s[:, j * 128:(j + 1) * 128]) * LOG2E
            w4d = wt.reshape(2, 8, 8, D)
            lo = _iota((8, D), 0) < 4
            parts, tails = [], []
            for gl in range(2):
                ref = w4d[gl, 7]
                f15 = jnp.where(lo, pltpu.roll(ref, 4, 0), ref)
                parts.append((w4d[gl, 0:7] - f15[None]).reshape(56, D))
                tails.append(ref - f15)
            pend += [tails[0] + pltpu.roll(tails[1], 4, 0)] + parts
            if j % 2 == 1:
                put_wT(row0 + (j - 1) * 120, jnp.concatenate(pend, axis=0).astype(BF))
                pend = []

    cp_wka.wait()
    start(grp_d)
    fold(wk_s, D, (0, 1))
    cp_wkb.wait()
    fold(wk_s, D, (2, 3))

    def main(_i, _c):
        pk, vt, xn1 = {}, {}, {}
        b1 = []
        phis = {}
        kvacc = [None] * G
        zacc = [None] * G

        def xblk(a):
            return xs[BND[a]:BND[a + 1], :]

        def do_pk(a):
            pk[a] = proj(D, PR, xblk(a))

        def do_v(a):
            vt[a] = proj(2 * D, D, xblk(a))

        def do_ln(c):
            v = _ln(xs[c * CH1:(c + 1) * CH1, :].astype(F32))
            xn1[c] = v if SW1 else v.astype(BF)

        def do_h(c):
            if c not in xn1:
                do_ln(c)
            if SW1:
                if not b1:
                    b1.extend(_prep(w1_s, NW1))
                h = _gelu(jnp.concatenate(_smm(_quads(xn1.pop(c)), b1), axis=0))
            else:
                h = _gelu(_dot(xn1.pop(c), w1_s[...]))
            r0 = c * CH1 + 8
            for g in range(4):
                hbuf[g, r0:r0 + CH1, :] = h[:, g * 128:(g + 1) * 128]

        def do_hs(a):
            for c in range(BND[a] // CH1, BND[a + 1] // CH1):
                do_h(c)

        def do_phi(a):
            if a in phis:
                return
            T = SZ[a]
            phis[a] = []
            p = pk.pop(a)
            for g in range(G):
                ep, en, sp, sn = _dual_exp(_group_rows(p, g))
                phi = jnp.concatenate([(ep * _rcp(sp)[None]).reshape(64, T),
                                       (en * _rcp(sn)[None]).reshape(64, T)], axis=0)
                zpart = phi[:, T - 128:]
                for l in range(T // 128 - 2, -1, -1):
                    zpart = zpart + phi[:, l * 128:(l + 1) * 128]
                zacc[g] = zpart if zacc[g] is None else zpart + zacc[g]
                phis[a].append(phi.astype(BF))

        def do_kv(a):
            do_phi(a)
            v = vt.pop(a)
            for g in range(G):
                kv = _dot_nt(v[g * 64:(g + 1) * 64, :].astype(BF), phis[a][g])
                kvacc[g] = kv if kvacc[g] is None else kvacc[g] + kv

        cp_xa.wait()
        for a in range(NA):
            do_pk(a)
            if a < NA - 1:
                do_phi(a)

        cp_xb.wait()
        start(grp_e)
        for a in range(NA, N0):
            do_pk(a)
            if a < N0 - 1:
                do_phi(a)
        do_ln(0)

        wait(grp_d)
        start(grp_f)
        put_wT(2 * D, wv_s[...].T)
        for a in range(N0):
            do_hs(a)
        for a in range(N0):
            do_v(a)
            do_kv(a)

        wait(grp_e)
        def do_fin(_):
            same_head = _iota((64, 128), 0) // DH == _iota((64, 128), 1) % 4
            for g in range(G):
                kvT[g] = jnp.where(same_head, kvacc[g], 0.0).astype(BF)
                zb[g] = jnp.broadcast_to(jnp.sum(zacc[g], axis=-1, keepdims=True), (128, 128))

        def do_prep(k):
            if k == 0 and PRE >= 1:
                _prep_store(c2, w2_s, D, step=PSTEP)
                _prep_store(co, wo_s, D, step=PSTEP)
            if k == 1 and PRE >= 2:
                wait(grp_f)
                _prep_store(c3, w3t_s, FM, transposed=True, step=PSTEP)
                _prep_store(c4, w4_s, FM, swap=True, step=PSTEP)

        fns = dict(p=do_pk, v=do_v, h=do_hs, k=do_kv, f=do_phi, z=do_fin, c=do_prep,
                   q=lambda _: fold(wq_s, 0, (0, 1, 2, 3)), H=do_h)
        for tok in SEG4.split(','):
            fns[tok[0]](int(tok[1:]))

        if PRE < 2:
            wait(grp_f)

        def p2(i, _):
            s0 = pl.multiple_of(i * TM2, TM2)
            gw = gate_s[...].astype(F32).reshape(1, D)

            if QPOS < 0:
                pqT = proj(0, PR, xs[pl.ds(s0, TM2), :])
            x1s, xns = [], []
            b2 = _prep_load(c2, NW2) if PRE >= 1 else _prep(w2_s, NW2)
            bo = _prep_load(co, NWO) if PRE >= 1 else _prep(wo_s, NWO)
            for c in range(TM2 // CH2):
                r0 = pl.multiple_of(s0 + c * CH2, CH2)
                hsh = jnp.concatenate([
                    hbuf[0, pl.ds(r0 + 7, CH2), :],
                    hbuf[1, pl.ds(r0 + 9, CH2), :],
                    hbuf[2, pl.ds(r0 + 6, CH2), :],
                    hbuf[3, pl.ds(r0 + 10, CH2), :]],
                    axis=1)
                if SW2:
                    hs = jnp.concatenate(_smm(_quads(hsh), b2), axis=0)
                else:
                    hs = _dot(hsh.astype(BF), w2_s[...])
                x1 = xs[pl.ds(r0, CH2), :].astype(F32) + (hs * GOUT if G5 else hs)
                x1s.append(x1)
                xns.append(_ln(x1))
            x1 = jnp.concatenate(x1s, axis=0)
            xn = jnp.concatenate(xns, axis=0)

            FH, KH, HR = FM // 2, D // 2, CH3 // 2
            b3 = {}
            for j in range(0, FH, NJ):
                w = min(NJ, FH - j)
                if PRE >= 2:
                    b3[j] = [pltpu.bitcast(c3[i, j // 2:(j + w) // 2, :], BF) for i in range(7)]
                    continue
                if WORDS:
                    ww = w3t_s.bitcast(jnp.uint32)
                    a0, a1, hw = j // 2, (FH + j) // 2, w // 2
                    b3[j] = _rhs7w(ww[a0:a0 + hw, 0:KH], ww[a1:a1 + hw, 0:KH],
                                   ww[a0:a0 + hw, KH:D], ww[a1:a1 + hw, KH:D])
                    continue
                b3[j] = _rhs7(w3t_s[j:j + w, 0:KH], w3t_s[FH + j:FH + j + w, 0:KH],
                              w3t_s[j:j + w, KH:D], w3t_s[FH + j:FH + j + w, KH:D])
            b4 = _prep_load(c4, NW4) if PRE >= 2 else _prep(w4_s, NW4, 0, FM, swap=True)
            l4s, yts = [], []
            zz = (one_s[0] - 1) * 8
            for c in range(TM2 // CH3):
                if c == QPOS:
                    pqT = proj(0, PR, xs[pl.ds(s0, TM2), :])
                xc = xn[c * CH3:(c + 1) * CH3]
                l3 = [v.astype(BF) for v in _lhs7(xc[:HR, :KH], xc[:HR, KH:],
                                                  xc[HR:, :KH], xc[HR:, KH:])]
                cols = [[] for _ in range(7)]
                for j in range(0, FH, NJ):
                    w = min(NJ, FH - j)
                    m = [None] * 7
                    for i in ORD3:
                        m[i] = _dot_nt(l3[i], b3[j][i])
                    y11, y12, y21, y22 = [_gelu(v) for v in _out4(m, ORD3)]
                    l7 = _lhs7(y12, y11, y22, y21) if SWAP else _lhs7(y11, y12, y21, y22)
                    if YB:
                        r = pl.multiple_of(zz + c * HR // 2, 8)
                        ybuf[j // NJ, pl.ds(r, HR // 2), :] = pltpu.bitcast(
                            jnp.concatenate(l7, axis=1).astype(BF), jnp.uint32)
                    else:
                        for i, v in enumerate(l7):
                            cols[i].append(v)
                if not YB:
                    l4s.append([jnp.concatenate(cc, axis=1) for cc in cols])
                yts.append(_gelu(_dot_nt(w3t_s[FM:F, :], xc.astype(BF))).T)
            if QPOS >= TM2 // CH3:
                pqT = proj(0, PR, xs[pl.ds(s0, TM2), :])

            oT = []
            for g in range(G):
                ep, en, sp, sn = _dual_exp(_group_rows(pqT, g))
                zt = jnp.concatenate([zb[g]] * (TM2 // 128), axis=1).reshape(2, 8, 8, TM2)
                rp = _rcp(sp)
                rn = _rcp(sn)
                den = _fold4(jnp.add, jnp.sum(ep * zt[0], axis=0) * rp
                             + jnp.sum(en * zt[1], axis=0) * rn) + 1e-6
                inv = _rcp(den)
                phi = jnp.concatenate([(ep * (rp * inv)[None]).reshape(64, TM2),
                                       (en * (rn * inv)[None]).reshape(64, TM2)], axis=0)
                oT.append(_dot(kvT[g], phi.astype(BF)))
            o = jnp.concatenate(oT, axis=0).T

            for c in range(TM2 // CH3):
                off = 0
                assert sum(OC[c]) == HR
                for n in OC[c]:
                    if TAILF:
                        tl = [_dot(yts[c][hh * HR + off:hh * HR + off + n].astype(BF),
                                   w4_s[FM:F, :]) for hh in range(2)]
                    hqs = _smm7([l4s[c][i][off:off + n].astype(BF) for i in range(7)], b4)
                    if SWO:
                        ot = o[c * CH3 + off:c * CH3 + off + n]
                        ob = o[c * CH3 + HR + off:c * CH3 + HR + off + n]
                        aa = _smm((ot[:, :KH], ot[:, KH:], ob[:, :KH], ob[:, KH:]), bo)
                    for half, hq in enumerate(hqs):
                        lo = half * HR + off
                        g0 = c * CH3 + lo
                        r0 = pl.multiple_of(s0 + g0, 16)
                        rows = slice(g0, g0 + n)
                        h2 = hq + (tl[half] if TAILF else
                                   _dot(yts[c][lo:lo + n].astype(BF), w4_s[FM:F, :]))
                        b = x1[rows] + (h2 * GOUT if G5 else h2)
                        a = aa[half] if SWO else _dot(o[rows].astype(BF), wo_s[...])
                        gl = jnp.sum(xs[pl.ds(r0, n), :].astype(F32) * gw, axis=-1,
                                     keepdims=True)
                        gate = 0.5 + 0.5 * jnp.tanh(0.5 * gl)
                        os_[pl.ds(r0, n), :] = (b + gate * (a - b)).astype(BF)
                        cp(os_.at[pl.ds(r0, n), :], o_hbm.at[pl.ds(r0, n), :],
                           out_sem).start()
                    off += n
            return 0

        jax.lax.fori_loop(0, S // TM2, p2, 0)
        return 0

    one_s[0] = 1
    jax.lax.fori_loop(0, one_s[0], main, 0)
    cp(os_, o_hbm, out_sem).wait()


def _compiler_params():
    base = dict(vmem_limit_bytes=100 * 2**20)
    try:
        return pltpu.CompilerParams(disable_bounds_checks=True,
                                    disable_semaphore_checks=True, **base)
    except TypeError:
        return pltpu.CompilerParams(**base)


@jax.jit
def pallas_gated_mix__linear_kernel_hedgehog__mixer_s_mlp__prompt_kernel(
    A_x: jax.Array,
    A_wqkv: jax.Array,
    A_w_phi: jax.Array,
    A_wo: jax.Array,
    B_x: jax.Array,
    B_w1: jax.Array,
    B_w2: jax.Array,
    B_w3: jax.Array,
    B_w4: jax.Array,
    gate_w: jax.Array,
):
    del B_x
    x = A_x.reshape(S, D)
    wphi = jnp.transpose(A_w_phi, (1, 2, 0)).reshape(DH * DH, H)
    hbm = pl.BlockSpec(memory_space=pl.ANY)
    out = pl.pallas_call(
        _kernel,
        out_shape=jax.ShapeDtypeStruct((S, D), BF),
        in_specs=[hbm] * 9,
        out_specs=hbm,
        scratch_shapes=[
            pltpu.VMEM((S, D), BF),
            pltpu.VMEM((D, D), BF),
            pltpu.VMEM((D, D), BF),
            pltpu.VMEM((D, D), BF),
            pltpu.VMEM((DH * DH, H), BF),
            pltpu.VMEM((D, D), BF),
            pltpu.VMEM((D, D), BF),
            pltpu.VMEM((D, D), BF),
            pltpu.VMEM((F, D), BF),
            pltpu.VMEM((F, D), BF),
            pltpu.VMEM((D,), BF),
            pltpu.VMEM((S, D), BF),
            pltpu.VMEM((3 * D // 2, D), jnp.uint32),
            pltpu.VMEM((4, S + 16, 128), F32),
            pltpu.VMEM((G, 64, 128), BF),
            pltpu.VMEM((G, 128, 128), F32),
            pltpu.VMEM((FM // 2 // NJ, TM2 // 4, 7 * NJ), jnp.uint32),
            pltpu.VMEM((7, D // 4, D // 2), jnp.uint32),
            pltpu.VMEM((7, D // 4, D // 2), jnp.uint32),
            pltpu.VMEM((7, FM // 4, D // 2), jnp.uint32),
            pltpu.VMEM((7, FM // 4, D // 2), jnp.uint32),
            pltpu.SMEM((1,), jnp.int32),
            pltpu.SemaphoreType.DMA((4,)),
        ],
        compiler_params=_compiler_params(),
    )(x, A_wqkv, wphi, A_wo, B_w1, B_w2, B_w3.T, B_w4, gate_w)
    return out.reshape(1, S, D)
```

```python
import math
import os

import jax
import jax.numpy as jnp
import jax.experimental.pallas as pl
import jax.experimental.pallas.tpu as pltpu

E = os.environ.get
S, D, H, DH, F = 2048, 512, 32, 16, 1376
G = 8
PR = 480
FM = 1280
FH, KH = FM // 2, D // 2
SZ = tuple(int(v) for v in E('SZ', '256,256,256,256,256,256,256,256').split(','))
BND = tuple(sum(SZ[:i]) for i in range(len(SZ) + 1))
NA, N0 = int(E('NA', 1)), int(E('N0', 3))
TM2 = 1024
CH1 = int(E('CH1', 128))
WC = [int(v) for v in E('WC', '128+128+128+128+128+128+128+128').split('+')]
FRESH = int(E('FRESH', 1))
SBQ = int(E('SBQ', 256))
OC = [int(v) for v in E('OC', '320+128+32+32').split('+')]
PAIRS = [int(v) for v in E('PAIRS', E('OC', '320+128+32+32')).split('+')]
POFF = [sum(PAIRS[:k]) for k in range(len(PAIRS))]
LNM = int(E('LNM', 1))
NH = int(E('NH', 1))
PIN = int(E('PIN', 0))
LNM1 = int(E('LNM1', 5))
ORD = [int(v) for v in E('ORD', '4213065')]
SW1 = int(E('SW1', 1))
SPQ = int(E('SPQ', 1))
RS = int(E('RS', 1))
BDT2 = int(E('BDT2', 0))
P1ONLY = int(E('P1ONLY', 0))
P2ONLY = int(E('P2ONLY', 0))
SEG2A = E('SEG2A', 'p0,e0')
SEG2B = E('SEG2B', 'p1,n0,p2,e2,f1')
SEG3 = E('SEG3', 'H0,v1,v0,H4,H3,H2,k0,v2,k2')
SEG4 = E('SEG4', 'p3,v3,H6,H8,H5,H7,p4,k3,v4,H9,p5,k4,v5,H10,k1,k5,p6,H1,v6,H15,H12,H11,H14,H13,q0,p7,v7,k6,k7,z0')
ORDER2 = E('ORDER2', 'W0,W1,W2,Q1,W3,W5,W7,Q0,Q2,Q3,W4,W6,T0,T3,T2,Y0,T4,N0,N1,T1,N2,N3,L2,F0,L0,L1,F1,O0,O1,F2,O2,L3,F3,O3')
LOG2E = math.log2(math.e)
GELU_C = math.sqrt(2.0 / math.pi)
GK = (GELU_C * 0.044715) ** (1.0 / 3.0)
GOUT = 0.5 / GK
BF = jnp.bfloat16
F32 = jnp.float32
NT = (((1,), (1,)), ((), ()))

_cur = []


def mark(name):
    if not int(E('SCOPES', 0)):
        return
    if _cur:
        _cur.pop().__exit__(None, None, None)
    if name:
        c = jax.named_scope(name)
        c.__enter__()
        _cur.append(c)


def _iota(shape, dim):
    return jax.lax.broadcasted_iota(jnp.int32, shape, dim)


def _dot(a, b):
    return jnp.dot(a, b, preferred_element_type=F32)


def _dot_nt(a, b):
    return jax.lax.dot_general(a, b, NT, preferred_element_type=F32)


def _lhs7(a11, a12, a21, a22):
    return [a11 + a22, a21 + a22, a11, a22, a11 + a12, a21 - a11, a12 - a22]


def _rhs7(b11, b12, b21, b22):
    f11, f12, f21, f22 = (b.astype(F32) for b in (b11, b12, b21, b22))
    return [(f11 + f22).astype(BF), b11, (f12 - f22).astype(BF), (f21 - f11).astype(BF),
            b22, (f11 + f12).astype(BF), (f21 + f22).astype(BF)]


def _rhs7_ref(ref, rows, cols, nr, nc, zero):
    cnt = [0]

    def ld(q):
        cnt[0] += 1
        r = rows[q] + zero * cnt[0] if FRESH else rows[q]
        if not isinstance(r, int):
            r = pl.multiple_of(r, 16)
        return ref[pl.ds(r, nr), cols[q]:cols[q] + nc]

    f = lambda q: ld(q).astype(F32)
    return [(f(0) + f(3)).astype(BF), ld(0), (f(1) - f(3)).astype(BF), (f(2) - f(0)).astype(BF),
            ld(3), (f(0) + f(1)).astype(BF), (f(2) + f(3)).astype(BF)]


_TERMS = (((0, 1), (3, 1), (4, -1), (6, 1)), ((2, 1), (4, 1)), ((1, 1), (3, 1)),
          ((0, 1), (1, -1), (2, 1), (5, 1)))


def _strassen(l7, b7, dot):
    m = [None] * 7
    for i in ORD:
        m[i] = dot(l7[i], b7[i])
    outs = []
    for terms in _TERMS:
        terms = sorted(terms, key=lambda t: -ORD.index(t[0]))
        assert terms[0][1] == 1
        acc = m[terms[0][0]]
        for i, sg in terms[1:]:
            acc = acc + m[i] if sg > 0 else acc - m[i]
        outs.append(acc)
    return outs


def _quads(a):
    h, k = a.shape[0] // 2, a.shape[1] // 2
    return a[:h, :k], a[:h, k:], a[h:, :k], a[h:, k:]


def _join(q):
    return jnp.concatenate([jnp.concatenate(q[:2], axis=1),
                            jnp.concatenate(q[2:], axis=1)], axis=0)


def _bf7(quads):
    return [v.astype(BF) for v in _lhs7(*quads)]


def _smm(a, b7):
    return _join(_strassen(_bf7(_quads(a)), b7, _dot))


def _gelu(y):
    return y + y * jnp.tanh(y * (GELU_C / GK + y * y))


def _ln(ld, mode):
    xf = ld()
    m = jnp.mean(xf, axis=-1, keepdims=True)
    if mode in (2, 5):
        v = jnp.maximum(jnp.mean(xf * xf, axis=-1, keepdims=True) - m * m, 0.0)
        xc = (ld() if mode == 5 else xf) - m
    else:
        xc = (ld() if mode in (4, 6) else xf) - m
        v = jnp.mean(xc * xc, axis=-1, keepdims=True)
    if RS:
        r = jnp.exp2(-0.5 * jnp.log2(v + 1e-5) + math.log2(GK))
    else:
        r = jax.lax.rsqrt(v * (1.0 / GK ** 2) + 1e-5 / GK ** 2)
    if mode == 1:
        return xf * r - m * r
    if mode in (3, 4):
        return (ld() - m) * r
    return xc * r


def _rcp(x):
    return pl.reciprocal(x, approx=True)


def _fold4(op, t):
    return op(t, pltpu.roll(t, 4, 0))


def _group_rows(pT, g):
    T = pT.shape[-1]
    base = (g // 2) * 120
    gl = g % 2
    x = pT[base: base + 8, :]
    body = pT[base + 8 + gl * 56: base + 8 + (gl + 1) * 56, :]
    lo = _iota((8, T), 0) < 4
    first = jnp.where(lo, x, 0.0) if gl == 0 else jnp.where(lo, 0.0, x)
    return jnp.concatenate([first, body], axis=0).reshape(8, 8, T)


def _dual_exp(p3):
    mx = _fold4(jnp.maximum, jnp.max(p3, axis=0))
    mn = _fold4(jnp.minimum, jnp.min(p3, axis=0))
    ep = jnp.exp2(p3 - mx[None])
    en = jnp.exp2(mn[None] - p3)
    sp = _fold4(jnp.add, jnp.sum(ep, axis=0))
    sn = _fold4(jnp.add, jnp.sum(en, axis=0))
    return ep, en, sp, sn


def _x7(load, T):
    h = T // 2
    return _rhs7(load(0, h, 0), load(h, h, 0), load(0, h, KH), load(h, h, KH))


def _kernel(x_hbm, wqkv_hbm, wphi_hbm, wo_hbm, w1_hbm, w2_hbm, w3t_hbm, w4_hbm, gate_hbm,
            o_hbm,
            xs, wq_s, wk_s, wv_s, wphi_s, wo_s, w1_s, w2_s, w3t_s, w4_s, gate_s, os_,
            wqT, lq7, hbuf, kvT, zb, one_s, sem):
    cp = pltpu.make_async_copy
    XA, X0 = BND[NA], BND[N0]
    cp_phi = cp(wphi_hbm, wphi_s, sem.at[0])
    cp_wka = cp(wqkv_hbm.at[:, D:D + KH], wk_s.at[:, 0:KH], sem.at[1])
    cp_wkb = cp(wqkv_hbm.at[:, D + KH:2 * D], wk_s.at[:, KH:D], sem.at[2])
    cp_xa = cp(x_hbm.at[0:XA, :], xs.at[0:XA, :], sem.at[3])
    cp_xb = cp(x_hbm.at[XA:X0, :], xs.at[XA:X0, :], sem.at[0])
    grp_d = [cp(w1_hbm, w1_s, sem.at[1]),
             cp(wqkv_hbm.at[:, 2 * D:3 * D], wv_s, sem.at[1])]
    grp_e = [cp(x_hbm.at[X0:S, :], xs.at[X0:S, :], sem.at[2]),
             cp(wqkv_hbm.at[:, 0:D], wq_s, sem.at[2])]
    grp_f = [cp(w2_hbm, w2_s, sem.at[3]),
             cp(w3t_hbm, w3t_s, sem.at[3]),
             cp(w4_hbm, w4_s, sem.at[3]),
             cp(wo_hbm, wo_s, sem.at[3]),
             cp(gate_hbm, gate_s, sem.at[3])]
    out_sem = sem.at[0]

    def start(grp):
        for c in grp:
            c.start()

    def wait(grp):
        for c in grp:
            c.wait()

    start([cp_phi, cp_wka, cp_wkb, cp_xa])

    for g in range(4):
        hbuf[g, 0:8, :] = jnp.zeros((8, 128), F32)
        hbuf[g, S + 8:S + 16, :] = jnp.zeros((8, 128), F32)

    mark('bdt')
    cp_phi.wait()
    cp_xb.start()
    if BDT2:
        wp = wphi_s[...].astype(F32)
        wp = jnp.concatenate([wp[q * 64:(q + 1) * 64] for q in range(4)], axis=1).astype(BF)
        kk, cc = _iota((128, D), 0), _iota((128, D), 1)
        sel = jnp.where((kk % H == cc // DH) & (kk // H == (cc % DH) // 4), 1.0, 0.0).astype(BF)
        t = _dot(wp, sel)
        t = jnp.where(_iota((64, D), 0) // DH == _iota((64, D), 1) % 4, t, 0.0).astype(BF)
        asel = jnp.where(_iota((64, 64), 0) // 4 == _iota((64, 64), 1) % DH, 1.0, 0.0).astype(BF)
    else:
        sel = jnp.where(_iota((H, D), 0) == _iota((H, D), 1) // DH, 1.0, 0.0).astype(BF)
        t = _dot(wphi_s[...], sel)
        t = jnp.where(_iota((256, D), 0) // DH == _iota((256, D), 1) % DH, t, 0.0).astype(BF)
        asel = jnp.where(_iota((64, 256), 0) // 4 == _iota((64, 256), 1) % DH,
                         1.0, 0.0).astype(BF)
    vrep = _dot(asel, t)
    hl = _iota((64, D), 0) % 4
    h8 = (_iota((64, D), 1) % 128) // DH
    bdt = jnp.concatenate([jnp.where(h8 == hl, vrep, 0.0),
                           jnp.where(h8 == hl + 4, vrep, 0.0)], axis=0).astype(BF)

    def fold(w_s, js):
        rows = []
        for j in js:
            wt = _dot_nt(bdt[:, j * 128:(j + 1) * 128], w_s[:, j * 128:(j + 1) * 128]) * LOG2E
            w4d = wt.reshape(2, 8, 8, D)
            lo = _iota((8, D), 0) < 4
            parts, tails = [], []
            for gl in range(2):
                ref = w4d[gl, 7]
                f15 = jnp.where(lo, pltpu.roll(ref, 4, 0), ref)
                parts.append((w4d[gl, 0:7] - f15[None]).reshape(56, D))
                tails.append(ref - f15)
            rows += [tails[0] + pltpu.roll(tails[1], 4, 0)] + parts
        return jnp.concatenate(rows, axis=0)

    mark('folda')
    cp_wka.wait()
    start(grp_d)
    kfa = fold(wk_s, (0, 1))
    mark('foldb')
    cp_wkb.wait()
    kfb = fold(wk_s, (2, 3))
    mark(None)

    def main(_i, _c):
        pk, vt, xn1, phis, ptile, xc7, lazy = {}, {}, {}, {}, {}, {}, {}
        kvacc = [None] * G
        zacc = [None] * G
        kf = jnp.concatenate([kfa, kfb], axis=0)
        zero = (one_s[0] - 1) * 16

        def pin(v):
            if PIN == 1:
                return pltpu.bitcast(pltpu.bitcast(v, jnp.int32) | zero, BF)
            if PIN == 2:
                return pltpu.bitcast(pltpu.bitcast(v, jnp.int32), BF)
            return v

        def once(key, fn):
            if key not in lazy:
                lazy[key] = fn()
            return lazy[key]

        def get_x7(b0, T):
            h = T // 2
            return once(('x7', b0, T), lambda: _rhs7_ref(
                xs, (b0, b0 + h, b0, b0 + h), (0, 0, KH, KH), h, KH, zero))

        def do_pk(a):
            if SZ[a] % 256 == 0:
                lk = once('lk', lambda: _bf7(_quads(kf)))
                pk[a] = _join(_strassen(lk, get_x7(BND[a], SZ[a]), _dot_nt))
            else:
                pk[a] = _dot_nt(once('kb', lambda: kf.astype(BF)), xs[BND[a]:BND[a + 1], :])

        def do_v(a):
            lv = once('lv', lambda: _bf7(_quads(wv_s[...].astype(F32).T)))
            T = SZ[a] if SZ[a] % 256 == 0 else SZ[a] + SZ[a + 1]
            v = _join(_strassen(lv, get_x7(BND[a], T), _dot_nt))
            vt[a] = v[:, :SZ[a]]
            if T != SZ[a]:
                vt[a + 1] = v[:, SZ[a]:]

        def do_ln(c):
            cnt = [0]

            def ld():
                cnt[0] += 1
                r = pl.multiple_of(c * CH1 + zero * (cnt[0] + 20), 16)
                return xs[pl.ds(r, CH1), :].astype(F32)

            v = _ln(ld, LNM1)
            xn1[c] = _bf7(_quads(v)) if SW1 else v.astype(BF)

        def do_h(c):
            if c not in xn1:
                do_ln(c)
            if SW1:
                b1 = once('b1', lambda: _rhs7_ref(w1_s, (0, 0, KH, KH), (0, KH, 0, KH), KH, KH, zero))
                h = _gelu(_join(_strassen(xn1.pop(c), b1, _dot)))
            else:
                h = _gelu(_dot(xn1.pop(c), w1_s[...]))
            r0 = c * CH1 + 8
            for g in range(4):
                hbuf[g, r0:r0 + CH1, :] = h[:, g * 128:(g + 1) * 128]

        def phi_tile(a, g, l):
            if (a, g, l) not in ptile:
                ep, en, sp, sn = _dual_exp(_group_rows(pk[a][:, l * 128:(l + 1) * 128], g))
                ptile[a, g, l] = jnp.concatenate(
                    [(ep * _rcp(sp)[None]).reshape(64, 128),
                     (en * _rcp(sn)[None]).reshape(64, 128)], axis=0)
            return ptile[a, g, l]

        def do_early(a):
            nt = SZ[a] // 128
            for g in range(G):
                for l in (range(nt // 2, nt) if g < 4 else range(nt // 2)):
                    phi_tile(a, g, l)

        def do_phi(a):
            if a in phis:
                return
            nt = SZ[a] // 128
            phis[a] = []
            for g in range(G):
                tiles = [phi_tile(a, g, l) for l in range(nt)]
                order = list(range(nt))
                if SZ[a] % 256 == 0 and g < 4:
                    order = order[nt // 2:] + order[:nt // 2]
                zpart = tiles[order[-1]]
                for l in reversed(order[:-1]):
                    zpart = zpart + tiles[l]
                zacc[g] = zpart if zacc[g] is None else zpart + zacc[g]
                phis[a].append(pin(jnp.concatenate(tiles, axis=1).astype(BF)))

        def do_kv(a):
            do_phi(a)
            v = vt[a]
            for g in range(G):
                kv = _dot_nt(v[g * 64:(g + 1) * 64, :].astype(BF), phis[a][g])
                kvacc[g] = kv if kvacc[g] is None else kv + kvacc[g]

        def do_fin(_):
            same_head = _iota((64, 128), 0) // DH == _iota((64, 128), 1) % 4
            for g in range(G):
                kvT[g] = jnp.where(same_head, kvacc[g], 0.0).astype(BF)
                zb[g] = jnp.broadcast_to(jnp.sum(zacc[g], axis=-1, keepdims=True), (128, 128))

        def do_fq(_):
            if SPQ == 1:
                qf = fold(wq_s, (0, 2, 1, 3))
                qf = jnp.concatenate([qf[0:120], qf[240:360], qf[120:240], qf[360:480]], axis=0)
                l7 = _lhs7(*_quads(qf))
                lq7[...] = pltpu.bitcast(jnp.concatenate(l7 + [l7[0]], axis=1).astype(BF),
                                         jnp.uint32)
            else:
                wqT[...] = pltpu.bitcast(fold(wq_s, (0, 1, 2, 3)).astype(BF), jnp.uint32)

        fns = dict(p=do_pk, v=do_v, k=do_kv, f=do_phi, z=do_fin, q=do_fq, H=do_h, n=do_ln,
                   e=do_early)

        def run(order):
            if P2ONLY:
                return
            for tok in order.split(','):
                fns[tok[0]](int(tok[1:]))

        mark('seg2')
        cp_xa.wait()
        run(SEG2A)
        mark('seg2b')
        cp_xb.wait()
        start(grp_e)
        run(SEG2B)
        mark('seg3')
        wait(grp_d)
        start(grp_f)
        run(SEG3)
        mark('seg4')
        wait(grp_e)
        run(SEG4)
        if P2ONLY:
            wqT[...] = pltpu.bitcast(kf.astype(BF), jnp.uint32)
        mark('p2')
        wait(grp_f)

        def p2(i, _):
            s0 = pl.multiple_of(i * TM2, TM2)
            gw = gate_s[...].astype(F32).reshape(1, D)
            st = {}
            offs = [sum(OC[:k]) for k in range(len(OC))]

            def lz(key, fn):
                if key not in st:
                    st[key] = fn()
                return st[key]

            def cat(name, n, axis=0):
                return lz(name, lambda: jnp.concatenate([st[name, c] for c in range(n)],
                                                        axis=axis))

            def do_w(c, plain=False):
                CH2 = WC[c]
                r0 = pl.multiple_of(s0 + sum(WC[:c]), 32)
                hsh = jnp.concatenate([
                    hbuf[0, pl.ds(r0 + 7, CH2), :],
                    hbuf[1, pl.ds(r0 + 9, CH2), :],
                    hbuf[2, pl.ds(r0 + 6, CH2), :],
                    hbuf[3, pl.ds(r0 + 10, CH2), :]],
                    axis=1)
                if plain:
                    hs = _dot(hsh.astype(BF), w2_s[...])
                else:
                    hs = _smm(hsh, lz('b2', lambda: _rhs7_ref(w2_s, (0, 0, KH, KH), (0, KH, 0, KH), KH, KH, zero)))
                x1 = xs[pl.ds(r0, CH2), :].astype(F32) + hs * GOUT
                st['x1', c] = x1
                st['xn', c] = _ln(lambda: x1, LNM)

            def do_q(t):
                t0 = t * SBQ
                if SPQ:
                    if SPQ == 1:
                        lq = [pltpu.bitcast(lq7[:, k * KH:(k + 1) * KH], BF) for k in range(7)]
                    else:
                        lq = lz('lq', lambda: _bf7(_quads(
                            pltpu.bitcast(wqT[...], BF).astype(F32))))
                    outs = []
                    for u in range(t0, t0 + SBQ, 256):
                        b0 = s0 + u
                        x7 = _rhs7_ref(xs, (b0, b0 + 128, b0, b0 + 128), (0, 0, KH, KH), 128,
                                       KH, zero)
                        outs.append(_join(_strassen(lq, x7, _dot_nt)))
                    st['pq', t] = jnp.concatenate(outs, axis=1)
                else:
                    st['pq', t] = _dot_nt(pltpu.bitcast(wqT[...], BF),
                                          xs[pl.ds(pl.multiple_of(s0 + t0, 128), SBQ), :])

            def split(v, lo, hi):
                top, bot = [], []
                for o, n in zip(POFF, PAIRS):
                    if lo <= o < hi:
                        r = 2 * (o - lo)
                        top.append(v[r:r + n])
                        bot.append(v[r + n:r + 2 * n])
                top, bot = jnp.concatenate(top, axis=0), jnp.concatenate(bot, axis=0)
                return top[:, :KH], top[:, KH:], bot[:, :KH], bot[:, KH:]

            def unsplit(q, lo, hi):
                top, bot = jnp.concatenate(q[:2], axis=1), jnp.concatenate(q[2:], axis=1)
                rows = []
                for o, n in zip(POFF, PAIRS):
                    if lo <= o < hi:
                        rows += [top[o - lo:o - lo + n], bot[o - lo:o - lo + n]]
                return jnp.concatenate(rows, axis=0)

            HS = TM2 // 2 // NH

            def rows_of(name, r0, n):
                parts, base, pos = [], None, 0
                for c, w in enumerate(WC):
                    if pos + w > r0 and pos < r0 + n:
                        if base is None:
                            base = pos
                        parts.append(st[name, c])
                    pos += w
                return jnp.concatenate(parts, axis=0)[r0 - base:r0 - base + n]

            def do_t(idx):
                sg, jj = divmod(idx, 5)
                j = jj * 128
                b3 = lz(('b3', jj), lambda: _rhs7_ref(
                    w3t_s, (j, FH + j, j, FH + j), (0, 0, KH, KH), 128, KH, zero))
                l3 = lz(('l3', sg), lambda: _bf7(
                    split(rows_of('xn', 2 * sg * HS, 2 * HS), sg * HS, (sg + 1) * HS)))
                y11, y12, y21, y22 = [_gelu(v) for v in _strassen(l3, b3, _dot_nt)]
                for k, v in enumerate(_lhs7(y12, y11, y22, y21)):
                    st[('l4', sg, k), jj] = v

            def do_y(sg):
                st['yt', sg] = _gelu(_dot_nt(
                    w3t_s[FM:F, :], rows_of('xn', 2 * sg * HS, 2 * HS).astype(BF))).T

            def do_n(t):
                pqT = st['pq', t]
                oT = []
                for g in range(G):
                    ep, en, sp, sn = _dual_exp(_group_rows(pqT, g))
                    zt = jnp.concatenate([zb[g]] * (SBQ // 128), axis=1).reshape(2, 8, 8, SBQ)
                    rp = _rcp(sp)
                    rn = _rcp(sn)
                    den = _fold4(jnp.add, jnp.sum(ep * zt[0], axis=0) * rp
                                 + jnp.sum(en * zt[1], axis=0) * rn) + 1e-6
                    inv = _rcp(den)
                    phi = jnp.concatenate([(ep * (rp * inv)[None]).reshape(64, SBQ),
                                           (en * (rn * inv)[None]).reshape(64, SBQ)], axis=0)
                    oT.append(_dot(kvT[g], pin(phi.astype(BF))))
                st['o', t] = jnp.concatenate(oT, axis=0).T

            def do_l(k):
                g0, n = 2 * offs[k], 2 * OC[k]
                sg = offs[k] // HS
                g0 -= 2 * sg * HS
                st['tl', k] = _dot(st['yt', sg][g0:g0 + n].astype(BF), w4_s[FM:F, :])

            def do_f(k):
                o_, n = offs[k], OC[k]
                b4 = lz('b4', lambda: _rhs7_ref(w4_s, (FH, FH, 0, 0), (0, KH, 0, KH), FH, KH,
                                                zero))
                sg = o_ // HS
                r = o_ - sg * HS
                l7 = [cat(('l4', sg, q), FH // 128, axis=1)[r:r + n].astype(BF)
                      for q in range(7)]
                st['h2', k] = unsplit(_strassen(l7, b4, _dot), o_, o_ + n)

            def do_o(k):
                g0, n = 2 * offs[k], 2 * OC[k]
                parts = [st['o', t] for t in range(g0 // SBQ, (g0 + n - 1) // SBQ + 1)]
                base = (g0 // SBQ) * SBQ
                o = jnp.concatenate(parts, axis=0)[g0 - base:g0 - base + n]
                bo = lz('bo', lambda: _rhs7_ref(wo_s, (0, 0, KH, KH), (0, KH, 0, KH), KH, KH, zero))
                lo, hi = offs[k], offs[k] + OC[k]
                a = unsplit(_strassen(_bf7(split(o, lo, hi)), bo, _dot), lo, hi)
                b = rows_of('x1', g0, n) + (st['h2', k] + st['tl', k]) * GOUT
                r0 = pl.multiple_of(s0 + g0, 16)
                gl = jnp.sum(xs[pl.ds(r0, n), :].astype(F32) * gw, axis=-1, keepdims=True)
                gate = 0.5 + 0.5 * jnp.tanh(0.5 * gl)
                os_[pl.ds(r0, n), :] = (b + gate * (a - b)).astype(BF)
                cp(os_.at[pl.ds(r0, n), :], o_hbm.at[pl.ds(r0, n), :], out_sem).start()

            f2 = dict(w=lambda c: do_w(c, True), W=do_w, Q=do_q, T=do_t, Y=do_y, N=do_n, L=do_l, F=do_f, O=do_o)
            for tok in ORDER2.split(','):
                f2[tok[0]](int(tok[1:]))
            return 0

        if P1ONLY:
            def p2s(i, _):
                w = lq7[0:64, 0:D] if SPQ == 1 else wqT[0:64, :]
                os_[pl.ds(i * 16, 16), :] = (
                    _dot(kvT[0][:16], pltpu.bitcast(w, BF))
                    + jnp.concatenate([zb[i, 0:16], hbuf[i, 0:16], hbuf[i, 16:32],
                                       kvT[i][:16].astype(F32)], axis=1)).astype(BF)
                return 0
            jax.lax.fori_loop(0, 2, p2s, 0)
            cp(os_, o_hbm, out_sem).start()
        else:
            jax.lax.fori_loop(0, S // TM2, p2, 0)
        mark(None)
        return 0

    one_s[0] = 1
    jax.lax.fori_loop(0, one_s[0], main, 0)
    mark('tail')
    cp(os_, o_hbm, out_sem).wait()
    mark(None)


def _compiler_params():
    base = dict(vmem_limit_bytes=100 * 2**20)
    try:
        return pltpu.CompilerParams(disable_bounds_checks=True,
                                    disable_semaphore_checks=True, **base)
    except TypeError:
        return pltpu.CompilerParams(**base)


@jax.jit
def pallas_gated_mix__linear_kernel_hedgehog__mixer_s_mlp__prompt_kernel(
    A_x, A_wqkv, A_w_phi, A_wo, B_x, B_w1, B_w2, B_w3, B_w4, gate_w):
    del B_x
    x = A_x.reshape(S, D)
    wphi = jnp.transpose(A_w_phi, (1, 2, 0)).reshape(DH * DH, H)
    hbm = pl.BlockSpec(memory_space=pl.ANY)
    out = pl.pallas_call(
        _kernel,
        out_shape=jax.ShapeDtypeStruct((S, D), BF),
        in_specs=[hbm] * 9,
        out_specs=hbm,
        scratch_shapes=[
            pltpu.VMEM((S, D), BF),
            pltpu.VMEM((D, D), BF),
            pltpu.VMEM((D, D), BF),
            pltpu.VMEM((D, D), BF),
            pltpu.VMEM((DH * DH, H), BF),
            pltpu.VMEM((D, D), BF),
            pltpu.VMEM((D, D), BF),
            pltpu.VMEM((D, D), BF),
            pltpu.VMEM((F, D), BF),
            pltpu.VMEM((F, D), BF),
            pltpu.VMEM((D,), BF),
            pltpu.VMEM((S, D), BF),
            pltpu.VMEM((PR // 2, D), jnp.uint32),
            pltpu.VMEM((PR // 4, 8 * KH), jnp.uint32),
            pltpu.VMEM((4, S + 16, 128), F32),
            pltpu.VMEM((G, 64, 128), BF),
            pltpu.VMEM((G, 128, 128), F32),
            pltpu.SMEM((1,), jnp.int32),
            pltpu.SemaphoreType.DMA((4,)),
        ],
        compiler_params=_compiler_params(),
    )(x, A_wqkv, wphi, A_wo, B_w1, B_w2, B_w3.T, B_w4, gate_w)
    return out.reshape(1, S, D)
```

```python
import math

import jax
import jax.numpy as jnp
import jax.experimental.pallas as pl
import jax.experimental.pallas.tpu as pltpu

S, D, H, DH, F = 2048, 512, 32, 16, 1376
G = 8
PR = 480
FM = 1280
FH, KH = FM // 2, D // 2
SB = 256
XA, XB = 256, 768
CH = 128
TM2 = 1024
OC = (320, 128, 32, 32)
OFF = tuple(sum(OC[:k]) for k in range(len(OC)))
SHIFT = (1, -1, 2, -2)

PHASE1 = ('p0,e0',
          'p1,n0,p2,e2,f1',
          'H0,v1,v0,H4,H3,H2,k0,v2,k2',
          'p3,v3,H6,H8,H5,H7,p4,k3,v4,H9,p5,k4,v5,H10,k1,k5,p6,H1,v6,H15,H12,H11,H14,H13,'
          'q0,p7,v7,k6,k7,z0')
PHASE2 = ('W0,W2,W1,W4,W3,W5,W6,W7,Q0,Q2,Q1,Q3,T0,T2,T1,T3,T4,N2,N1,N0,Y0,'
          'F0,N3,L1,L0,F1,O0,O1,L2,F2,O2,L3,F3,O3')

LOG2E = math.log2(math.e)
GELU_C = math.sqrt(2.0 / math.pi)
GK = (GELU_C * 0.044715) ** (1.0 / 3.0)
GOUT = 0.5 / GK
BF = jnp.bfloat16
F32 = jnp.float32
NT = (((1,), (1,)), ((), ()))


def _iota(shape, dim):
    return jax.lax.broadcasted_iota(jnp.int32, shape, dim)


def _dot(a, b):
    return jnp.dot(a, b, preferred_element_type=F32)


def _dot_nt(a, b):
    return jax.lax.dot_general(a, b, NT, preferred_element_type=F32)


def _lhs7(a11, a12, a21, a22):
    return [a11 + a22, a21 + a22, a11, a22, a11 + a12, a21 - a11, a12 - a22]


def _rhs7(ref, rows, cols, nr, nc, zero):
    cnt = [0]

    def ld(q):
        cnt[0] += 1
        r = pl.multiple_of(rows[q] + zero * cnt[0], 16)
        return ref[pl.ds(r, nr), cols[q]:cols[q] + nc]

    def f(q):
        return ld(q).astype(F32)

    return [(f(0) + f(3)).astype(BF), ld(0), (f(1) - f(3)).astype(BF), (f(2) - f(0)).astype(BF),
            ld(3), (f(0) + f(1)).astype(BF), (f(2) + f(3)).astype(BF)]


_TERMS = (((0, 1), (3, 1), (4, -1), (6, 1)), ((2, 1), (4, 1)), ((1, 1), (3, 1)),
          ((0, 1), (1, -1), (2, 1), (5, 1)))


def _strassen(l7, b7, dot, order='4213065'):
    order = [int(c) for c in order]
    m = [None] * 7
    for i in order:
        m[i] = dot(l7[i], b7[i])
    outs = []
    for terms in _TERMS:
        terms = sorted(terms, key=lambda t: -order.index(t[0]))
        if terms[0][1] < 0:
            acc = m[terms[1][0]] - m[terms[0][0]]
            terms = terms[1:]
        else:
            acc = m[terms[0][0]]
        for i, sign in terms[1:]:
            acc = acc + m[i] if sign > 0 else acc - m[i]
        outs.append(acc)
    return outs


def _quads(a):
    h, k = a.shape[0] // 2, a.shape[1] // 2
    return a[:h, :k], a[:h, k:], a[h:, :k], a[h:, k:]


def _join(q):
    return jnp.concatenate([jnp.concatenate(q[:2], axis=1),
                            jnp.concatenate(q[2:], axis=1)], axis=0)


def _bf7(quads):
    return [v.astype(BF) for v in _lhs7(*quads)]


def _gelu(y):
    return y + y * jnp.tanh(y * (GELU_C / GK + y * y))


def _inv_std(v):
    return jnp.exp2(-0.5 * jnp.log2(v + 1e-5) + math.log2(GK))


def _rcp(x):
    return pl.reciprocal(x, approx=True)


def _fold4(op, t):
    return op(t, pltpu.roll(t, 4, 0))


def _group_rows(pT, g):
    T = pT.shape[-1]
    base = (g // 2) * 120
    gl = g % 2
    x = pT[base: base + 8, :]
    body = pT[base + 8 + gl * 56: base + 8 + (gl + 1) * 56, :]
    lo = _iota((8, T), 0) < 4
    first = jnp.where(lo, x, 0.0) if gl == 0 else jnp.where(lo, 0.0, x)
    return jnp.concatenate([first, body], axis=0).reshape(8, 8, T)


def _dual_exp(p3):
    mx = _fold4(jnp.maximum, jnp.max(p3, axis=0))
    mn = _fold4(jnp.minimum, jnp.min(p3, axis=0))
    ep = jnp.exp2(p3 - mx[None])
    en = jnp.exp2(mn[None] - p3)
    sp = _fold4(jnp.add, jnp.sum(ep, axis=0))
    sn = _fold4(jnp.add, jnp.sum(en, axis=0))
    return ep, en, sp, sn


def _run(fns, order):
    for tok in order.split(','):
        fns[tok[0]](int(tok[1:]))


def _kernel(x_hbm, wqkv_hbm, wphi_hbm, wo_hbm, w1_hbm, w2_hbm, w3t_hbm, w4_hbm, gate_hbm,
            o_hbm,
            xs, wq_s, wk_s, wv_s, wphi_s, wo_s, w1_s, w2_s, w3t_s, w4_s, gate_s, os_,
            wqT, hbuf, kvT, zb, one_s, sem):
    cp = pltpu.make_async_copy
    cp_phi = cp(wphi_hbm, wphi_s, sem.at[0])
    cp_wka = cp(wqkv_hbm.at[:, D:D + KH], wk_s.at[:, 0:KH], sem.at[1])
    cp_wkb = cp(wqkv_hbm.at[:, D + KH:2 * D], wk_s.at[:, KH:D], sem.at[2])
    cp_xa = cp(x_hbm.at[0:XA, :], xs.at[0:XA, :], sem.at[3])
    cp_xb = cp(x_hbm.at[XA:XB, :], xs.at[XA:XB, :], sem.at[0])
    grp_d = [cp(w1_hbm, w1_s, sem.at[1]),
             cp(wqkv_hbm.at[:, 2 * D:3 * D], wv_s, sem.at[1])]
    grp_e = [cp(x_hbm.at[XB:S, :], xs.at[XB:S, :], sem.at[2]),
             cp(wqkv_hbm.at[:, 0:D], wq_s, sem.at[2])]
    grp_f = [cp(w2_hbm, w2_s, sem.at[3]),
             cp(w3t_hbm, w3t_s, sem.at[3]),
             cp(w4_hbm, w4_s, sem.at[3]),
             cp(wo_hbm, wo_s, sem.at[3]),
             cp(gate_hbm, gate_s, sem.at[3])]
    out_sem = sem.at[0]

    def start(grp):
        for c in grp:
            c.start()

    def wait(grp):
        for c in grp:
            c.wait()

    start([cp_phi, cp_wka, cp_wkb, cp_xa])

    for g in range(4):
        hbuf[g, 8:16, :] = jnp.zeros((8, 128), F32)
        hbuf[g, S:S + 8, :] = jnp.zeros((8, 128), F32)

    cp_phi.wait()
    cp_xb.start()
    sel = jnp.where(_iota((H, D), 0) == _iota((H, D), 1) // DH, 1.0, 0.0).astype(BF)
    t = _dot(wphi_s[...], sel)
    t = jnp.where(_iota((256, D), 0) // DH == _iota((256, D), 1) % DH, t, 0.0).astype(BF)
    asel = jnp.where(_iota((64, 256), 0) // 4 == _iota((64, 256), 1) % DH, 1.0, 0.0).astype(BF)
    vrep = _dot(asel, t)
    hl = _iota((64, D), 0) % 4
    h8 = (_iota((64, D), 1) % 128) // DH
    bdt = jnp.concatenate([jnp.where(h8 == hl, vrep, 0.0),
                           jnp.where(h8 == hl + 4, vrep, 0.0)], axis=0).astype(BF)

    def fold(w_s, js):
        rows = []
        for j in js:
            wt = _dot_nt(bdt[:, j * 128:(j + 1) * 128], w_s[:, j * 128:(j + 1) * 128]) * LOG2E
            w4d = wt.reshape(2, 8, 8, D)
            lo = _iota((8, D), 0) < 4
            parts, tails = [], []
            for gl in range(2):
                ref = w4d[gl, 7]
                f15 = jnp.where(lo, pltpu.roll(ref, 4, 0), ref)
                parts.append((w4d[gl, 0:7] - f15[None]).reshape(56, D))
                tails.append(ref - f15)
            rows += [tails[0] + pltpu.roll(tails[1], 4, 0)] + parts
        return jnp.concatenate(rows, axis=0)

    cp_wka.wait()
    start(grp_d)
    kfa = fold(wk_s, (0, 1))
    cp_wkb.wait()
    kfb = fold(wk_s, (2, 3))

    def main(_i, _c):
        zero = (one_s[0] - 1) * 16
        square = ((0, 0, KH, KH), (0, KH, 0, KH), KH, KH, zero)

        pk, vt, xn1, phis, ptile, lazy = {}, {}, {}, {}, {}, {}
        kvacc = [None] * G
        zacc = [None] * G

        def once(key, fn):
            if key not in lazy:
                lazy[key] = fn()
            return lazy[key]

        def x7(a):
            b0, h = a * SB, SB // 2
            return once(('x7', a), lambda: _rhs7(
                xs, (b0, b0 + h, b0, b0 + h), (0, 0, KH, KH), h, KH, zero))

        def do_pk(a):
            lk = once('lk', lambda: _bf7(_quads(jnp.concatenate([kfa, kfb], axis=0))))
            pk[a] = _join(_strassen(lk, x7(a), _dot_nt))

        def do_v(a):
            lv = once('lv', lambda: _bf7(_quads(wv_s[...].astype(F32).T)))
            vt[a] = _join(_strassen(lv, x7(a), _dot_nt))

        def do_ln(c):
            def ld(k):
                r = pl.multiple_of(c * CH + zero * k, 16)
                return xs[pl.ds(r, CH), :].astype(F32)

            xf = ld(21)
            m = jnp.mean(xf, axis=-1, keepdims=True)
            v = jnp.maximum(jnp.mean(xf * xf, axis=-1, keepdims=True) - m * m, 0.0)
            xn1[c] = _bf7(_quads((ld(22) - m) * _inv_std(v)))

        def do_h(c):
            if c not in xn1:
                do_ln(c)
            b1 = once('b1', lambda: _rhs7(w1_s, *square))
            h = _gelu(_join(_strassen(xn1.pop(c), b1, _dot)))
            for g in range(4):
                r = c * CH + 8 + SHIFT[g]
                hbuf[g, r:r + CH, :] = h[:, g * 128:(g + 1) * 128]

        def phi_tile(a, g, l):
            if (a, g, l) not in ptile:
                ep, en, sp, sn = _dual_exp(_group_rows(pk[a][:, l * 128:(l + 1) * 128], g))
                ptile[a, g, l] = jnp.concatenate(
                    [(ep * _rcp(sp)[None]).reshape(64, 128),
                     (en * _rcp(sn)[None]).reshape(64, 128)], axis=0)
            return ptile[a, g, l]

        def do_early(a):
            for g in range(G):
                phi_tile(a, g, 1 if g < 4 else 0)

        def do_phi(a):
            if a in phis:
                return
            phis[a] = []
            for g in range(G):
                tiles = [phi_tile(a, g, l) for l in range(2)]
                zpart = tiles[0] + tiles[1] if g < 4 else tiles[1] + tiles[0]
                zacc[g] = zpart if zacc[g] is None else zpart + zacc[g]
                phis[a].append(jnp.concatenate(tiles, axis=1).astype(BF))

        def do_kv(a):
            do_phi(a)
            for g in range(G):
                kv = _dot_nt(vt[a][g * 64:(g + 1) * 64, :].astype(BF), phis[a][g])
                kvacc[g] = kv if kvacc[g] is None else kv + kvacc[g]

        def do_fin(_):
            same_head = _iota((64, 128), 0) // DH == _iota((64, 128), 1) % 4
            for g in range(G):
                kvT[g] = jnp.where(same_head, kvacc[g], 0.0).astype(BF)
                zb[g] = jnp.broadcast_to(jnp.sum(zacc[g], axis=-1, keepdims=True), (128, 128))

        def do_fq(_):
            wqT[...] = pltpu.bitcast(fold(wq_s, (0, 1, 2, 3)).astype(BF), jnp.uint32)

        f1 = dict(p=do_pk, v=do_v, k=do_kv, f=do_phi, z=do_fin, q=do_fq, H=do_h, n=do_ln,
                  e=do_early)
        cp_xa.wait()
        _run(f1, PHASE1[0])
        cp_xb.wait()
        start(grp_e)
        _run(f1, PHASE1[1])
        wait(grp_d)
        start(grp_f)
        _run(f1, PHASE1[2])
        wait(grp_e)
        _run(f1, PHASE1[3])
        wait(grp_f)

        def p2(i, _):
            s0 = pl.multiple_of(i * TM2, TM2)
            gw = gate_s[...].astype(F32).reshape(1, D)
            st = {}

            def lz(key, fn):
                if key not in st:
                    st[key] = fn()
                return st[key]

            def rows_of(name, size, r0, n):
                c0, c1 = r0 // size, (r0 + n - 1) // size + 1
                v = jnp.concatenate([st[name, c] for c in range(c0, c1)], axis=0)
                return v[r0 - c0 * size:r0 - c0 * size + n]

            def do_w(c):
                r0 = pl.multiple_of(s0 + c * CH, 32)
                hsh = jnp.concatenate([hbuf[g, pl.ds(r0 + 8, CH), :] for g in range(4)], axis=1)
                b2 = lz('b2', lambda: _rhs7(w2_s, *square))
                hs = _join(_strassen(_bf7(_quads(hsh)), b2, _dot, '1024365'))
                x1 = xs[pl.ds(r0, CH), :].astype(F32) + hs * GOUT
                m = jnp.mean(x1, axis=-1, keepdims=True)
                xc = x1 - m
                r = _inv_std(jnp.mean(xc * xc, axis=-1, keepdims=True))
                st['x1', c] = x1
                st['xn', c] = x1 * r - m * r

            def do_q(t):
                st['pq', t] = _dot_nt(pltpu.bitcast(wqT[...], BF),
                                      xs[pl.ds(pl.multiple_of(s0 + t * SB, 128), SB), :])

            def l3():
                xn = rows_of('xn', CH, 0, TM2)
                top = jnp.concatenate([xn[2 * o:2 * o + n] for o, n in zip(OFF, OC)], axis=0)
                bot = jnp.concatenate([xn[2 * o + n:2 * o + 2 * n] for o, n in zip(OFF, OC)],
                                      axis=0)
                return _bf7((top[:, :KH], top[:, KH:], bot[:, :KH], bot[:, KH:]))

            def do_t(jj):
                j = jj * 128
                b3 = _rhs7(w3t_s, (j, FH + j, j, FH + j), (0, 0, KH, KH), 128, KH, zero)
                y11, y12, y21, y22 = [
                    _gelu(v) for v in _strassen(lz('l3', l3), b3, _dot_nt, '4213605')]
                st['l4', jj] = _lhs7(y12, y11, y22, y21)

            def do_y(_):
                st['yt'] = _gelu(
                    _dot_nt(w3t_s[FM:F, :], rows_of('xn', CH, 0, TM2).astype(BF))).T

            def do_n(t):
                oT = []
                for g in range(G):
                    ep, en, sp, sn = _dual_exp(_group_rows(st['pq', t], g))
                    zt = jnp.concatenate([zb[g]] * (SB // 128), axis=1).reshape(2, 8, 8, SB)
                    rp = _rcp(sp)
                    rn = _rcp(sn)
                    den = _fold4(jnp.add, jnp.sum(ep * zt[0], axis=0) * rp
                                 + jnp.sum(en * zt[1], axis=0) * rn) + 1e-6
                    inv = _rcp(den)
                    phi = jnp.concatenate([(ep * (rp * inv)[None]).reshape(64, SB),
                                           (en * (rn * inv)[None]).reshape(64, SB)], axis=0)
                    oT.append(_dot(kvT[g], phi.astype(BF)))
                st['o', t] = jnp.concatenate(oT, axis=0).T

            def do_l(k):
                g0, n = 2 * OFF[k], 2 * OC[k]
                st['tl', k] = _dot(st['yt'][g0:g0 + n].astype(BF), w4_s[FM:F, :])

            def do_f(k):
                b4 = lz('b4', lambda: _rhs7(w4_s, (FH, FH, 0, 0), (0, KH, 0, KH), FH, KH, zero))
                l4 = lz('l4', lambda: [
                    jnp.concatenate([st['l4', jj][q] for jj in range(FH // 128)], axis=1)
                    for q in range(7)])
                l7 = [v[OFF[k]:OFF[k] + OC[k]].astype(BF) for v in l4]
                st['h2', k] = _join(_strassen(l7, b4, _dot, '4321065'))

            def do_o(k):
                g0, n = 2 * OFF[k], 2 * OC[k]
                bo = lz('bo', lambda: _rhs7(wo_s, *square))
                a = _join(_strassen(_bf7(_quads(rows_of('o', SB, g0, n))), bo, _dot, '0143265'))
                b = rows_of('x1', CH, g0, n) + (st['h2', k] + st['tl', k]) * GOUT
                r0 = pl.multiple_of(s0 + g0, 16)
                gl = jnp.sum(xs[pl.ds(r0, n), :].astype(F32) * gw, axis=-1, keepdims=True)
                gate = 0.5 + 0.5 * jnp.tanh(0.5 * gl)
                res = (b + gate * (a - b)).astype(BF)
                parts = 2 if k == len(OC) - 1 else 1
                m = n // parts
                for u in range(parts):
                    r = pl.multiple_of(r0 + u * m, 16)
                    os_[pl.ds(r, m), :] = res[u * m:(u + 1) * m]
                    cp(os_.at[pl.ds(r, m), :], o_hbm.at[pl.ds(r, m), :], out_sem).start()

            _run(dict(W=do_w, Q=do_q, T=do_t, Y=do_y, N=do_n, L=do_l, F=do_f, O=do_o), PHASE2)
            return 0

        jax.lax.fori_loop(0, S // TM2, p2, 0)
        return 0

    one_s[0] = 1
    jax.lax.fori_loop(0, one_s[0], main, 0)
    cp(os_, o_hbm, out_sem).wait()


def _compiler_params():
    base = dict(vmem_limit_bytes=100 * 2**20)
    try:
        return pltpu.CompilerParams(disable_bounds_checks=True,
                                    disable_semaphore_checks=True, **base)
    except TypeError:
        return pltpu.CompilerParams(**base)


@jax.jit
def pallas_gated_mix__linear_kernel_hedgehog__mixer_s_mlp__prompt_kernel(
    A_x: jax.Array,
    A_wqkv: jax.Array,
    A_w_phi: jax.Array,
    A_wo: jax.Array,
    B_x: jax.Array,
    B_w1: jax.Array,
    B_w2: jax.Array,
    B_w3: jax.Array,
    B_w4: jax.Array,
    gate_w: jax.Array,
):
    del B_x
    x = A_x.reshape(S, D)
    wphi = jnp.transpose(A_w_phi, (1, 2, 0)).reshape(DH * DH, H)
    hbm = pl.BlockSpec(memory_space=pl.ANY)
    out = pl.pallas_call(
        _kernel,
        out_shape=jax.ShapeDtypeStruct((S, D), BF),
        in_specs=[hbm] * 9,
        out_specs=hbm,
        scratch_shapes=[
            pltpu.VMEM((S, D), BF),
            pltpu.VMEM((D, D), BF),
            pltpu.VMEM((D, D), BF),
            pltpu.VMEM((D, D), BF),
            pltpu.VMEM((DH * DH, H), BF),
            pltpu.VMEM((D, D), BF),
            pltpu.VMEM((D, D), BF),
            pltpu.VMEM((D, D), BF),
            pltpu.VMEM((F, D), BF),
            pltpu.VMEM((F, D), BF),
            pltpu.VMEM((D,), BF),
            pltpu.VMEM((S, D), BF),
            pltpu.VMEM((PR // 2, D), jnp.uint32),
            pltpu.VMEM((4, S + 16, 128), F32),
            pltpu.VMEM((G, 64, 128), BF),
            pltpu.VMEM((G, 128, 128), F32),
            pltpu.SMEM((1,), jnp.int32),
            pltpu.SemaphoreType.DMA((4,)),
        ],
        compiler_params=_compiler_params(),
    )(x, A_wqkv, wphi, A_wo, B_w1, B_w2, B_w3.T, B_w4, gate_w)
    return out.reshape(1, S, D)
```

```python
import math

import jax
import jax.numpy as jnp
import jax.experimental.pallas as pl
import jax.experimental.pallas.tpu as pltpu

S, D, H, DH, F = 2048, 512, 32, 16, 1376
G = 8
PR = 480
FM = 1280
FH, KH = FM // 2, D // 2
SB = 256
XA, XB = 256, 768
CH = 128
TM2 = 1024
OC = (320, 128, 32, 32)
OFF = tuple(sum(OC[:k]) for k in range(len(OC)))
SHIFT = (1, -1, 2, -2)

PHASE1 = ('p0,e0',
          'p1,n0,p2,e2,f1',
          'H0,v1,v0,H4,H3,H2,k0,v2,k2',
          'p3,v3,H6,H8,H5,H7,p4,k3,v4,H9,p5,k4,v5,H10,k1,k5,p6,H1,v6,H15,H12,H11,H14,H13,'
          'q0,p7,v7,k6,k7,z0')
PHASE2 = ('W0,W2,W1,W4,W3,W5,W6,W7,Q0,Q2,Q1,Q3,T0,T2,T1,T3,T4,N2,N1,N0,Y0,'
          'F0,N3,L1,L0,F1,O0,O1,L2,F2,O2,L3,F3,O3')

LOG2E = math.log2(math.e)
GELU_C = math.sqrt(2.0 / math.pi)
GK = (GELU_C * 0.044715) ** (1.0 / 3.0)
GOUT = 0.5 / GK
BF = jnp.bfloat16
F32 = jnp.float32
NT = (((1,), (1,)), ((), ()))


def _iota(shape, dim):
    return jax.lax.broadcasted_iota(jnp.int32, shape, dim)


def _dot(a, b):
    return jnp.dot(a, b, preferred_element_type=F32)


def _dot_nt(a, b):
    return jax.lax.dot_general(a, b, NT, preferred_element_type=F32)


def _lhs7(a11, a12, a21, a22):
    return [a11 + a22, a21 + a22, a11, a22, a11 + a12, a21 - a11, a12 - a22]


def _rhs7(ref, rows, cols, nr, nc, zero):
    cnt = [0]

    def ld(q):
        cnt[0] += 1
        r = pl.multiple_of(rows[q] + zero * cnt[0], 16)
        return ref[pl.ds(r, nr), cols[q]:cols[q] + nc]

    def f(q):
        return ld(q).astype(F32)

    return [(f(0) + f(3)).astype(BF), ld(0), (f(1) - f(3)).astype(BF), (f(2) - f(0)).astype(BF),
            ld(3), (f(0) + f(1)).astype(BF), (f(2) + f(3)).astype(BF)]


_TERMS = (((0, 1), (3, 1), (4, -1), (6, 1)), ((2, 1), (4, 1)), ((1, 1), (3, 1)),
          ((0, 1), (1, -1), (2, 1), (5, 1)))


def _strassen(l7, b7, dot, order='4213065'):
    order = [int(c) for c in order]
    m = [None] * 7
    for i in order:
        m[i] = dot(l7[i], b7[i])
    outs = []
    for terms in _TERMS:
        terms = sorted(terms, key=lambda t: -order.index(t[0]))
        if terms[0][1] < 0:
            acc = m[terms[1][0]] - m[terms[0][0]]
            terms = terms[1:]
        else:
            acc = m[terms[0][0]]
        for i, sign in terms[1:]:
            acc = acc + m[i] if sign > 0 else acc - m[i]
        outs.append(acc)
    return outs


def _quads(a):
    h, k = a.shape[0] // 2, a.shape[1] // 2
    return a[:h, :k], a[:h, k:], a[h:, :k], a[h:, k:]


def _join(q):
    return jnp.concatenate([jnp.concatenate(q[:2], axis=1),
                            jnp.concatenate(q[2:], axis=1)], axis=0)


def _bf7(quads):
    return [v.astype(BF) for v in _lhs7(*quads)]


def _gelu(y):
    return y + y * jnp.tanh(y * (GELU_C / GK + y * y))


def _inv_std(v):
    return jnp.exp2(-0.5 * jnp.log2(v + 1e-5) + math.log2(GK))


def _rcp(x):
    return pl.reciprocal(x, approx=True)


def _fold4(op, t):
    return op(t, pltpu.roll(t, 4, 0))


def _group_rows(pT, g):
    T = pT.shape[-1]
    base = (g // 2) * 120
    gl = g % 2
    x = pT[base: base + 8, :]
    body = pT[base + 8 + gl * 56: base + 8 + (gl + 1) * 56, :]
    lo = _iota((8, T), 0) < 4
    first = jnp.where(lo, x, 0.0) if gl == 0 else jnp.where(lo, 0.0, x)
    return jnp.concatenate([first, body], axis=0).reshape(8, 8, T)


def _dual_exp(p3):
    mx = _fold4(jnp.maximum, jnp.max(p3, axis=0))
    mn = _fold4(jnp.minimum, jnp.min(p3, axis=0))
    ep = jnp.exp2(p3 - mx[None])
    en = jnp.exp2(mn[None] - p3)
    sp = _fold4(jnp.add, jnp.sum(ep, axis=0))
    sn = _fold4(jnp.add, jnp.sum(en, axis=0))
    return ep, en, sp, sn


def _run(fns, order):
    for tok in order.split(','):
        fns[tok[0]](int(tok[1:]))


def _kernel(x_hbm, wqkv_hbm, wphi_hbm, wo_hbm, w1_hbm, w2_hbm, w3t_hbm, w4_hbm, gate_hbm,
            o_hbm,
            xs, wq_s, wk_s, wv_s, wphi_s, wo_s, w1_s, w2_s, w3t_s, w4_s, gate_s, os_,
            wqT, hbuf, kvT, zb, sem):
    cp = pltpu.make_async_copy
    cp_phi = cp(wphi_hbm, wphi_s, sem.at[0])
    cp_wka = cp(wqkv_hbm.at[:, D:D + KH], wk_s.at[:, 0:KH], sem.at[1])
    cp_wkb = cp(wqkv_hbm.at[:, D + KH:2 * D], wk_s.at[:, KH:D], sem.at[2])
    cp_xa = cp(x_hbm.at[0:XA, :], xs.at[0:XA, :], sem.at[3])
    cp_xb = cp(x_hbm.at[XA:XB, :], xs.at[XA:XB, :], sem.at[0])
    grp_d = [cp(w1_hbm, w1_s, sem.at[1]),
             cp(wqkv_hbm.at[:, 2 * D:3 * D], wv_s, sem.at[1])]
    grp_e = [cp(x_hbm.at[XB:S, :], xs.at[XB:S, :], sem.at[2]),
             cp(wqkv_hbm.at[:, 0:D], wq_s, sem.at[2])]
    grp_f = [cp(w2_hbm, w2_s, sem.at[3]),
             cp(w3t_hbm, w3t_s, sem.at[3]),
             cp(w4_hbm, w4_s, sem.at[3]),
             cp(wo_hbm, wo_s, sem.at[3]),
             cp(gate_hbm, gate_s, sem.at[3])]
    out_sem = sem.at[0]

    def start(grp):
        for c in grp:
            c.start()

    def wait(grp):
        for c in grp:
            c.wait()

    start([cp_phi, cp_wka, cp_wkb, cp_xa])

    for g in range(4):
        hbuf[g, 8:16, :] = jnp.zeros((8, 128), F32)
        hbuf[g, S:S + 8, :] = jnp.zeros((8, 128), F32)

    cp_phi.wait()
    cp_xb.start()
    sel = jnp.where(_iota((H, D), 0) == _iota((H, D), 1) // DH, 1.0, 0.0).astype(BF)
    t = _dot(wphi_s[...], sel)
    t = jnp.where(_iota((256, D), 0) // DH == _iota((256, D), 1) % DH, t, 0.0).astype(BF)
    asel = jnp.where(_iota((64, 256), 0) // 4 == _iota((64, 256), 1) % DH, 1.0, 0.0).astype(BF)
    vrep = _dot(asel, t)
    hl = _iota((64, D), 0) % 4
    h8 = (_iota((64, D), 1) % 128) // DH
    bdt = jnp.concatenate([jnp.where(h8 == hl, vrep, 0.0),
                           jnp.where(h8 == hl + 4, vrep, 0.0)], axis=0).astype(BF)

    def fold(w_s, js):
        rows = []
        for j in js:
            wt = _dot_nt(bdt[:, j * 128:(j + 1) * 128], w_s[:, j * 128:(j + 1) * 128]) * LOG2E
            w4d = wt.reshape(2, 8, 8, D)
            lo = _iota((8, D), 0) < 4
            parts, tails = [], []
            for gl in range(2):
                ref = w4d[gl, 7]
                f15 = jnp.where(lo, pltpu.roll(ref, 4, 0), ref)
                parts.append((w4d[gl, 0:7] - f15[None]).reshape(56, D))
                tails.append(ref - f15)
            rows += [tails[0] + pltpu.roll(tails[1], 4, 0)] + parts
        return jnp.concatenate(rows, axis=0)

    cp_wka.wait()
    start(grp_d)
    kfa = fold(wk_s, (0, 1))
    cp_wkb.wait()
    kfb = fold(wk_s, (2, 3))

    def main(_i, _c):
        zero = pl.program_id(0) * 16
        square = ((0, 0, KH, KH), (0, KH, 0, KH), KH, KH, zero)

        pk, vt, xn1, phis, ptile, lazy = {}, {}, {}, {}, {}, {}
        kvacc = [None] * G
        zacc = [None] * G

        def once(key, fn):
            if key not in lazy:
                lazy[key] = fn()
            return lazy[key]

        def x7(a):
            b0, h = a * SB, SB // 2
            return once(('x7', a), lambda: _rhs7(
                xs, (b0, b0 + h, b0, b0 + h), (0, 0, KH, KH), h, KH, zero))

        def do_pk(a):
            lk = once('lk', lambda: _bf7(_quads(jnp.concatenate([kfa, kfb], axis=0))))
            pk[a] = _join(_strassen(lk, x7(a), _dot_nt))

        def do_v(a):
            lv = once('lv', lambda: _bf7(_quads(wv_s[...].astype(F32).T)))
            vt[a] = _join(_strassen(lv, x7(a), _dot_nt))

        def do_ln(c):
            def ld(k):
                r = pl.multiple_of(c * CH + zero * k, 16)
                return xs[pl.ds(r, CH), :].astype(F32)

            xf = ld(21)
            m = jnp.mean(xf, axis=-1, keepdims=True)
            v = jnp.maximum(jnp.mean(xf * xf, axis=-1, keepdims=True) - m * m, 0.0)
            xn1[c] = _bf7(_quads((ld(22) - m) * _inv_std(v)))

        def do_h(c):
            if c not in xn1:
                do_ln(c)
            b1 = once('b1', lambda: _rhs7(w1_s, *square))
            h = _gelu(_join(_strassen(xn1.pop(c), b1, _dot)))
            for g in range(4):
                r = c * CH + 8 + SHIFT[g]
                hbuf[g, r:r + CH, :] = h[:, g * 128:(g + 1) * 128]

        def phi_tile(a, g, l):
            if (a, g, l) not in ptile:
                ep, en, sp, sn = _dual_exp(_group_rows(pk[a][:, l * 128:(l + 1) * 128], g))
                ptile[a, g, l] = jnp.concatenate(
                    [(ep * _rcp(sp)[None]).reshape(64, 128),
                     (en * _rcp(sn)[None]).reshape(64, 128)], axis=0)
            return ptile[a, g, l]

        def do_early(a):
            for g in range(G):
                phi_tile(a, g, 1 if g < 4 else 0)

        def do_phi(a):
            if a in phis:
                return
            phis[a] = []
            for g in range(G):
                tiles = [phi_tile(a, g, l) for l in range(2)]
                zpart = tiles[0] + tiles[1] if g < 4 else tiles[1] + tiles[0]
                zacc[g] = zpart if zacc[g] is None else zpart + zacc[g]
                phis[a].append(jnp.concatenate(tiles, axis=1).astype(BF))

        def do_kv(a):
            do_phi(a)
            for g in range(G):
                kv = _dot_nt(vt[a][g * 64:(g + 1) * 64, :].astype(BF), phis[a][g])
                kvacc[g] = kv if kvacc[g] is None else kv + kvacc[g]

        def do_fin(_):
            same_head = _iota((64, 128), 0) // DH == _iota((64, 128), 1) % 4
            for g in range(G):
                kvT[g] = jnp.where(same_head, kvacc[g], 0.0).astype(BF)
                zb[g] = jnp.broadcast_to(jnp.sum(zacc[g], axis=-1, keepdims=True), (128, 128))

        def do_fq(_):
            wqT[...] = pltpu.bitcast(fold(wq_s, (0, 1, 2, 3)).astype(BF), jnp.uint32)

        f1 = dict(p=do_pk, v=do_v, k=do_kv, f=do_phi, z=do_fin, q=do_fq, H=do_h, n=do_ln,
                  e=do_early)
        cp_xa.wait()
        _run(f1, PHASE1[0])
        cp_xb.wait()
        start(grp_e)
        _run(f1, PHASE1[1])
        wait(grp_d)
        start(grp_f)
        _run(f1, PHASE1[2])
        wait(grp_e)
        _run(f1, PHASE1[3])
        wait(grp_f)

        def p2(i, _):
            s0 = pl.multiple_of(i * TM2, TM2)
            gw = gate_s[...].astype(F32).reshape(1, D)
            st = {}

            def lz(key, fn):
                if key not in st:
                    st[key] = fn()
                return st[key]

            def rows_of(name, size, r0, n):
                c0, c1 = r0 // size, (r0 + n - 1) // size + 1
                v = jnp.concatenate([st[name, c] for c in range(c0, c1)], axis=0)
                return v[r0 - c0 * size:r0 - c0 * size + n]

            def do_w(c):
                r0 = pl.multiple_of(s0 + c * CH, 32)
                hsh = jnp.concatenate([hbuf[g, pl.ds(r0 + 8, CH), :] for g in range(4)], axis=1)
                b2 = lz('b2', lambda: _rhs7(w2_s, *square))
                hs = _join(_strassen(_bf7(_quads(hsh)), b2, _dot, '1024365'))
                x1 = xs[pl.ds(r0, CH), :].astype(F32) + hs * GOUT
                m = jnp.mean(x1, axis=-1, keepdims=True)
                xc = x1 - m
                r = _inv_std(jnp.mean(xc * xc, axis=-1, keepdims=True))
                st['x1', c] = x1
                st['xn', c] = x1 * r - m * r

            def do_q(t):
                st['pq', t] = _dot_nt(pltpu.bitcast(wqT[...], BF),
                                      xs[pl.ds(pl.multiple_of(s0 + t * SB, 128), SB), :])

            def l3():
                xn = rows_of('xn', CH, 0, TM2)
                top = jnp.concatenate([xn[2 * o:2 * o + n] for o, n in zip(OFF, OC)], axis=0)
                bot = jnp.concatenate([xn[2 * o + n:2 * o + 2 * n] for o, n in zip(OFF, OC)],
                                      axis=0)
                return _bf7((top[:, :KH], top[:, KH:], bot[:, :KH], bot[:, KH:]))

            def do_t(jj):
                j = jj * 128
                b3 = _rhs7(w3t_s, (j, FH + j, j, FH + j), (0, 0, KH, KH), 128, KH, zero)
                y11, y12, y21, y22 = [
                    _gelu(v) for v in _strassen(lz('l3', l3), b3, _dot_nt, '4213605')]
                st['l4', jj] = _lhs7(y12, y11, y22, y21)

            def do_y(_):
                st['yt'] = _gelu(
                    _dot_nt(w3t_s[FM:F, :], rows_of('xn', CH, 0, TM2).astype(BF))).T

            def do_n(t):
                oT = []
                for g in range(G):
                    ep, en, sp, sn = _dual_exp(_group_rows(st['pq', t], g))
                    zt = jnp.concatenate([zb[g]] * (SB // 128), axis=1).reshape(2, 8, 8, SB)
                    rp = _rcp(sp)
                    rn = _rcp(sn)
                    den = _fold4(jnp.add, jnp.sum(ep * zt[0], axis=0) * rp
                                 + jnp.sum(en * zt[1], axis=0) * rn) + 1e-6
                    inv = _rcp(den)
                    phi = jnp.concatenate([(ep * (rp * inv)[None]).reshape(64, SB),
                                           (en * (rn * inv)[None]).reshape(64, SB)], axis=0)
                    oT.append(_dot(kvT[g], phi.astype(BF)))
                st['o', t] = jnp.concatenate(oT, axis=0).T

            def do_l(k):
                g0, n = 2 * OFF[k], 2 * OC[k]
                st['tl', k] = _dot(st['yt'][g0:g0 + n].astype(BF), w4_s[FM:F, :])

            def do_f(k):
                b4 = lz('b4', lambda: _rhs7(w4_s, (FH, FH, 0, 0), (0, KH, 0, KH), FH, KH, zero))
                l4 = lz('l4', lambda: [
                    jnp.concatenate([st['l4', jj][q] for jj in range(FH // 128)], axis=1)
                    for q in range(7)])
                l7 = [v[OFF[k]:OFF[k] + OC[k]].astype(BF) for v in l4]
                st['h2', k] = _join(_strassen(l7, b4, _dot, '4321065'))

            def do_o(k):
                g0, n = 2 * OFF[k], 2 * OC[k]
                bo = lz('bo', lambda: _rhs7(wo_s, *square))
                a = _join(_strassen(_bf7(_quads(rows_of('o', SB, g0, n))), bo, _dot, '0143265'))
                b = rows_of('x1', CH, g0, n) + (st['h2', k] + st['tl', k]) * GOUT
                r0 = pl.multiple_of(s0 + g0, 16)
                gl = jnp.sum(xs[pl.ds(r0, n), :].astype(F32) * gw, axis=-1, keepdims=True)
                gate = 0.5 + 0.5 * jnp.tanh(0.5 * gl)
                res = (b + gate * (a - b)).astype(BF)
                parts = 2 if k == len(OC) - 1 else 1
                m = n // parts
                for u in range(parts):
                    r = pl.multiple_of(r0 + u * m, 16)
                    os_[pl.ds(r, m), :] = res[u * m:(u + 1) * m]
                    cp(os_.at[pl.ds(r, m), :], o_hbm.at[pl.ds(r, m), :], out_sem).start()

            _run(dict(W=do_w, Q=do_q, T=do_t, Y=do_y, N=do_n, L=do_l, F=do_f, O=do_o), PHASE2)
            return 0

        jax.lax.fori_loop(0, S // TM2, p2, 0)
        return 0

    jax.lax.fori_loop(0, pl.program_id(0) + 1, main, 0)
    cp(os_, o_hbm, out_sem).wait()


def _compiler_params():
    base = dict(vmem_limit_bytes=100 * 2**20)
    try:
        return pltpu.CompilerParams(disable_bounds_checks=True,
                                    disable_semaphore_checks=True, **base)
    except TypeError:
        return pltpu.CompilerParams(**base)


@jax.jit
def pallas_gated_mix__linear_kernel_hedgehog__mixer_s_mlp__prompt_kernel(
    A_x: jax.Array,
    A_wqkv: jax.Array,
    A_w_phi: jax.Array,
    A_wo: jax.Array,
    B_x: jax.Array,
    B_w1: jax.Array,
    B_w2: jax.Array,
    B_w3: jax.Array,
    B_w4: jax.Array,
    gate_w: jax.Array,
):
    del B_x
    x = A_x.reshape(S, D)
    wphi = jnp.transpose(A_w_phi, (1, 2, 0)).reshape(DH * DH, H)
    hbm = pl.BlockSpec(memory_space=pl.ANY)
    out = pl.pallas_call(
        _kernel,
        out_shape=jax.ShapeDtypeStruct((S, D), BF),
        grid=(1,),
        in_specs=[hbm] * 9,
        out_specs=hbm,
        scratch_shapes=[
            pltpu.VMEM((S, D), BF),
            pltpu.VMEM((D, D), BF),
            pltpu.VMEM((D, D), BF),
            pltpu.VMEM((D, D), BF),
            pltpu.VMEM((DH * DH, H), BF),
            pltpu.VMEM((D, D), BF),
            pltpu.VMEM((D, D), BF),
            pltpu.VMEM((D, D), BF),
            pltpu.VMEM((F, D), BF),
            pltpu.VMEM((F, D), BF),
            pltpu.VMEM((D,), BF),
            pltpu.VMEM((S, D), BF),
            pltpu.VMEM((PR // 2, D), jnp.uint32),
            pltpu.VMEM((4, S + 16, 128), F32),
            pltpu.VMEM((G, 64, 128), BF),
            pltpu.VMEM((G, 128, 128), F32),
            pltpu.SemaphoreType.DMA((4,)),
        ],
        compiler_params=_compiler_params(),
    )(x, A_wqkv, wphi, A_wo, B_w1, B_w2, B_w3.T, B_w4, gate_w)
    return out.reshape(1, S, D)
```

```python
import math

import jax
import jax.numpy as jnp
import jax.experimental.pallas as pl
import jax.experimental.pallas.tpu as pltpu

S, D, H, DH, F = 2048, 512, 32, 16, 1376
G = 8
PR = 480
FM = 1280
FH, KH = FM // 2, D // 2
SB = 256
XA, XB = 256, 768
CH = 128
TM2 = 1024
OC = (320, 128, 32, 32)
OFF = tuple(sum(OC[:k]) for k in range(len(OC)))
SHIFT = (1, -1, 2, -2)

PHASE1 = ('p0,e0',
          'p1,f1,p2,e2,n0',
          'H0,v0,v1,H4,H2,k0,v2,k2',
          'p3,v3,H6,H7,H8,H5,p4,k3,v4,H9,p5,v5,H10,k4,p6,H1,v6,H3,k1,k5,H14,H12,H11,H15,'
          'q0,H13,p7,v7,k6,k7,z0')
PHASE2 = ('W0,W2,W6,W1,W4,W3,W5,W7,Q0,Q2,Q1,Q3,T0,T2,T3,T1,T4,N2,N1,N0,Y0,'
          'F0,N3,L1,L0,F1,O0,O1,L3,L2,F2,O2,F3,O3')

LOG2E = math.log2(math.e)
GELU_C = math.sqrt(2.0 / math.pi)
GK = (GELU_C * 0.044715) ** (1.0 / 3.0)
GOUT = 0.5 / GK
BF = jnp.bfloat16
F32 = jnp.float32
NT = (((1,), (1,)), ((), ()))


def _iota(shape, dim):
    return jax.lax.broadcasted_iota(jnp.int32, shape, dim)


def _dot(a, b):
    return jnp.dot(a, b, preferred_element_type=F32)


def _dot_nt(a, b):
    return jax.lax.dot_general(a, b, NT, preferred_element_type=F32)


def _lhs7(a11, a12, a21, a22):
    return [a11 + a22, a21 + a22, a11, a22, a11 + a12, a21 - a11, a12 - a22]


def _rhs7(ref, rows, cols, nr, nc, zero):
    cnt = [0]

    def ld(q):
        cnt[0] += 1
        r = pl.multiple_of(rows[q] + zero * cnt[0], 16)
        return ref[pl.ds(r, nr), cols[q]:cols[q] + nc]

    def f(q):
        return ld(q).astype(F32)

    return [(f(0) + f(3)).astype(BF), ld(0), (f(1) - f(3)).astype(BF), (f(2) - f(0)).astype(BF),
            ld(3), (f(0) + f(1)).astype(BF), (f(2) + f(3)).astype(BF)]


_TERMS = (((0, 1), (3, 1), (4, -1), (6, 1)), ((2, 1), (4, 1)), ((1, 1), (3, 1)),
          ((0, 1), (1, -1), (2, 1), (5, 1)))


def _strassen(l7, b7, dot, order='4213065'):
    order = [int(c) for c in order]
    m = [None] * 7
    for i in order:
        m[i] = dot(l7[i], b7[i])
    outs = []
    for terms in _TERMS:
        terms = sorted(terms, key=lambda t: -order.index(t[0]))
        if terms[0][1] < 0:
            acc = m[terms[1][0]] - m[terms[0][0]]
            terms = terms[1:]
        else:
            acc = m[terms[0][0]]
        for i, sign in terms[1:]:
            acc = acc + m[i] if sign > 0 else acc - m[i]
        outs.append(acc)
    return outs


def _quads(a):
    h, k = a.shape[0] // 2, a.shape[1] // 2
    return a[:h, :k], a[:h, k:], a[h:, :k], a[h:, k:]


def _join(q):
    return jnp.concatenate([jnp.concatenate(q[:2], axis=1),
                            jnp.concatenate(q[2:], axis=1)], axis=0)


def _bf7(quads):
    return [v.astype(BF) for v in _lhs7(*quads)]


def _gelu(y):
    return y + y * jnp.tanh(y * (GELU_C / GK + y * y))


def _inv_std(v):
    return jnp.exp2(-0.5 * jnp.log2(v + 1e-5) + math.log2(GK))


def _rcp(x):
    return pl.reciprocal(x, approx=True)


def _fold4(op, t):
    return op(t, pltpu.roll(t, 4, 0))


def _group_rows(pT, g):
    T = pT.shape[-1]
    base = (g // 2) * 120
    gl = g % 2
    x = pT[base: base + 8, :]
    body = pT[base + 8 + gl * 56: base + 8 + (gl + 1) * 56, :]
    lo = _iota((8, T), 0) < 4
    first = jnp.where(lo, x, 0.0) if gl == 0 else jnp.where(lo, 0.0, x)
    return jnp.concatenate([first, body], axis=0).reshape(8, 8, T)


def _dual_exp(p3):
    mx = _fold4(jnp.maximum, jnp.max(p3, axis=0))
    mn = _fold4(jnp.minimum, jnp.min(p3, axis=0))
    ep = jnp.exp2(p3 - mx[None])
    en = jnp.exp2(mn[None] - p3)
    sp = _fold4(jnp.add, jnp.sum(ep, axis=0))
    sn = _fold4(jnp.add, jnp.sum(en, axis=0))
    return ep, en, sp, sn


def _run(fns, order):
    for tok in order.split(','):
        fns[tok[0]](int(tok[1:]))


def _kernel(x_hbm, wqkv_hbm, wphi_hbm, wo_hbm, w1_hbm, w2_hbm, w3t_hbm, w4_hbm, gate_hbm,
            o_hbm,
            xs, wq_s, wk_s, wv_s, wphi_s, wo_s, w1_s, w2_s, w3t_s, w4_s, gate_s, os_,
            wqT, hbuf, kvT, zb, sem):
    cp = pltpu.make_async_copy
    cp_phi = cp(wphi_hbm, wphi_s, sem.at[0])
    cp_wka = cp(wqkv_hbm.at[:, D:D + KH], wk_s.at[:, 0:KH], sem.at[1])
    cp_wkb = cp(wqkv_hbm.at[:, D + KH:2 * D], wk_s.at[:, KH:D], sem.at[2])
    cp_xa = cp(x_hbm.at[0:XA, :], xs.at[0:XA, :], sem.at[3])
    cp_xb = cp(x_hbm.at[XA:XB, :], xs.at[XA:XB, :], sem.at[0])
    grp_d = [cp(w1_hbm, w1_s, sem.at[1]),
             cp(wqkv_hbm.at[:, 2 * D:3 * D], wv_s, sem.at[1])]
    grp_e = [cp(x_hbm.at[XB:S, :], xs.at[XB:S, :], sem.at[2]),
             cp(wqkv_hbm.at[:, 0:D], wq_s, sem.at[2])]
    grp_f = [cp(w2_hbm, w2_s, sem.at[3]),
             cp(w3t_hbm, w3t_s, sem.at[3]),
             cp(w4_hbm, w4_s, sem.at[3]),
             cp(wo_hbm, wo_s, sem.at[3]),
             cp(gate_hbm, gate_s, sem.at[3])]
    out_sem = sem.at[0]

    def start(grp):
        for c in grp:
            c.start()

    def wait(grp):
        for c in grp:
            c.wait()

    start([cp_phi, cp_wka, cp_wkb, cp_xa])

    for g in range(4):
        hbuf[g, 8:16, :] = jnp.zeros((8, 128), F32)
        hbuf[g, S:S + 8, :] = jnp.zeros((8, 128), F32)

    cp_phi.wait()
    cp_xb.start()
    sel = jnp.where(_iota((H, D), 0) == _iota((H, D), 1) // DH, 1.0, 0.0).astype(BF)
    t = _dot(wphi_s[...], sel)
    t = jnp.where(_iota((256, D), 0) // DH == _iota((256, D), 1) % DH, t, 0.0).astype(BF)
    asel = jnp.where(_iota((64, 256), 0) // 4 == _iota((64, 256), 1) % DH, 1.0, 0.0).astype(BF)
    vrep = _dot(asel, t)
    hl = _iota((64, D), 0) % 4
    h8 = (_iota((64, D), 1) % 128) // DH
    bdt = jnp.concatenate([jnp.where(h8 == hl, vrep, 0.0),
                           jnp.where(h8 == hl + 4, vrep, 0.0)], axis=0).astype(BF)

    def fold(w_s, js):
        rows = []
        for j in js:
            wt = _dot_nt(bdt[:, j * 128:(j + 1) * 128], w_s[:, j * 128:(j + 1) * 128]) * LOG2E
            w4d = wt.reshape(2, 8, 8, D)
            lo = _iota((8, D), 0) < 4
            parts, tails = [], []
            for gl in range(2):
                ref = w4d[gl, 7]
                f15 = jnp.where(lo, pltpu.roll(ref, 4, 0), ref)
                parts.append((w4d[gl, 0:7] - f15[None]).reshape(56, D))
                tails.append(ref - f15)
            rows += [tails[0] + pltpu.roll(tails[1], 4, 0)] + parts
        return jnp.concatenate(rows, axis=0)

    cp_wka.wait()
    start(grp_d)
    kfa = fold(wk_s, (0, 1))
    cp_wkb.wait()
    kfb = fold(wk_s, (2, 3))

    def main(_i, _c):
        zero = pl.program_id(0) * 16
        square = ((0, 0, KH, KH), (0, KH, 0, KH), KH, KH, zero)

        pk, vt, xn1, phis, ptile, lazy = {}, {}, {}, {}, {}, {}
        kvacc = [None] * G
        zacc = [None] * G

        def once(key, fn):
            if key not in lazy:
                lazy[key] = fn()
            return lazy[key]

        def x7(a):
            b0, h = a * SB, SB // 2
            return once(('x7', a), lambda: _rhs7(
                xs, (b0, b0 + h, b0, b0 + h), (0, 0, KH, KH), h, KH, zero))

        def do_pk(a):
            lk = once('lk', lambda: _bf7(_quads(jnp.concatenate([kfa, kfb], axis=0))))
            pk[a] = _join(_strassen(lk, x7(a), _dot_nt))

        def do_v(a):
            lv = once('lv', lambda: _bf7(_quads(wv_s[...].astype(F32).T)))
            vt[a] = _join(_strassen(lv, x7(a), _dot_nt))

        def do_ln(c):
            def ld(k):
                r = pl.multiple_of(c * CH + zero * k, 16)
                return xs[pl.ds(r, CH), :].astype(F32)

            xf = ld(21)
            m = jnp.mean(xf, axis=-1, keepdims=True)
            v = jnp.maximum(jnp.mean(xf * xf, axis=-1, keepdims=True) - m * m, 0.0)
            xn1[c] = _bf7(_quads((ld(22) - m) * _inv_std(v)))

        def do_h(c):
            if c not in xn1:
                do_ln(c)
            b1 = once('b1', lambda: _rhs7(w1_s, *square))
            h = _gelu(_join(_strassen(xn1.pop(c), b1, _dot)))
            for g in range(4):
                r = c * CH + 8 + SHIFT[g]
                hbuf[g, r:r + CH, :] = h[:, g * 128:(g + 1) * 128]

        def phi_tile(a, g, l):
            if (a, g, l) not in ptile:
                ep, en, sp, sn = _dual_exp(_group_rows(pk[a][:, l * 128:(l + 1) * 128], g))
                ptile[a, g, l] = jnp.concatenate(
                    [(ep * _rcp(sp)[None]).reshape(64, 128),
                     (en * _rcp(sn)[None]).reshape(64, 128)], axis=0)
            return ptile[a, g, l]

        def do_early(a):
            for g in range(G):
                phi_tile(a, g, 1 if g < 4 else 0)

        def do_phi(a):
            if a in phis:
                return
            phis[a] = []
            for g in range(G):
                tiles = [phi_tile(a, g, l) for l in range(2)]
                zpart = tiles[0] + tiles[1] if g < 4 else tiles[1] + tiles[0]
                zacc[g] = zpart if zacc[g] is None else zpart + zacc[g]
                phis[a].append(jnp.concatenate(tiles, axis=1).astype(BF))

        def do_kv(a):
            do_phi(a)
            for g in range(G):
                kv = _dot_nt(vt[a][g * 64:(g + 1) * 64, :].astype(BF), phis[a][g])
                kvacc[g] = kv if kvacc[g] is None else kv + kvacc[g]

        def do_fin(_):
            same_head = _iota((64, 128), 0) // DH == _iota((64, 128), 1) % 4
            for g in range(G):
                kvT[g] = jnp.where(same_head, kvacc[g], 0.0).astype(BF)
                zb[g] = jnp.broadcast_to(jnp.sum(zacc[g], axis=-1, keepdims=True), (128, 128))

        def do_fq(_):
            wqT[...] = pltpu.bitcast(fold(wq_s, (0, 1, 2, 3)).astype(BF), jnp.uint32)

        f1 = dict(p=do_pk, v=do_v, k=do_kv, f=do_phi, z=do_fin, q=do_fq, H=do_h, n=do_ln,
                  e=do_early)
        cp_xa.wait()
        _run(f1, PHASE1[0])
        cp_xb.wait()
        start(grp_e)
        _run(f1, PHASE1[1])
        wait(grp_d)
        start(grp_f)
        _run(f1, PHASE1[2])
        wait(grp_e)
        _run(f1, PHASE1[3])
        wait(grp_f)

        def p2(i, _):
            s0 = pl.multiple_of(i * TM2, TM2)
            gw = gate_s[...].astype(F32).reshape(1, D)
            st = {}

            def lz(key, fn):
                if key not in st:
                    st[key] = fn()
                return st[key]

            def rows_of(name, size, r0, n):
                c0, c1 = r0 // size, (r0 + n - 1) // size + 1
                v = jnp.concatenate([st[name, c] for c in range(c0, c1)], axis=0)
                return v[r0 - c0 * size:r0 - c0 * size + n]

            def do_w(c):
                r0 = pl.multiple_of(s0 + c * CH, 32)
                hsh = jnp.concatenate([hbuf[g, pl.ds(r0 + 8, CH), :] for g in range(4)], axis=1)
                b2 = lz('b2', lambda: _rhs7(w2_s, *square))
                hs = _join(_strassen(_bf7(_quads(hsh)), b2, _dot, '1024365'))
                x1 = xs[pl.ds(r0, CH), :].astype(F32) + hs * GOUT
                m = jnp.mean(x1, axis=-1, keepdims=True)
                xc = x1 - m
                r = _inv_std(jnp.mean(xc * xc, axis=-1, keepdims=True))
                st['x1', c] = x1
                st['xn', c] = x1 * r - m * r

            def do_q(t):
                st['pq', t] = _dot_nt(pltpu.bitcast(wqT[...], BF),
                                      xs[pl.ds(pl.multiple_of(s0 + t * SB, 128), SB), :])

            def l3():
                xn = rows_of('xn', CH, 0, TM2)
                top = jnp.concatenate([xn[2 * o:2 * o + n] for o, n in zip(OFF, OC)], axis=0)
                bot = jnp.concatenate([xn[2 * o + n:2 * o + 2 * n] for o, n in zip(OFF, OC)],
                                      axis=0)
                return _bf7((top[:, :KH], top[:, KH:], bot[:, :KH], bot[:, KH:]))

            def do_t(jj):
                j = jj * 128
                b3 = _rhs7(w3t_s, (j, FH + j, j, FH + j), (0, 0, KH, KH), 128, KH, zero)
                y11, y12, y21, y22 = [
                    _gelu(v) for v in _strassen(lz('l3', l3), b3, _dot_nt, '4213605')]
                st['l4', jj] = _lhs7(y12, y11, y22, y21)

            def do_y(_):
                st['yt'] = _gelu(
                    _dot_nt(w3t_s[FM:F, :], rows_of('xn', CH, 0, TM2).astype(BF))).T

            def do_n(t):
                oT = []
                for g in range(G):
                    ep, en, sp, sn = _dual_exp(_group_rows(st['pq', t], g))
                    zt = jnp.concatenate([zb[g]] * (SB // 128), axis=1).reshape(2, 8, 8, SB)
                    rp = _rcp(sp)
                    rn = _rcp(sn)
                    den = _fold4(jnp.add, jnp.sum(ep * zt[0], axis=0) * rp
                                 + jnp.sum(en * zt[1], axis=0) * rn) + 1e-6
                    inv = _rcp(den)
                    phi = jnp.concatenate([(ep * (rp * inv)[None]).reshape(64, SB),
                                           (en * (rn * inv)[None]).reshape(64, SB)], axis=0)
                    oT.append(_dot(kvT[g], phi.astype(BF)))
                st['o', t] = jnp.concatenate(oT, axis=0).T

            def do_l(k):
                g0, n = 2 * OFF[k], 2 * OC[k]
                st['tl', k] = _dot(st['yt'][g0:g0 + n].astype(BF), w4_s[FM:F, :])

            def do_f(k):
                b4 = lz('b4', lambda: _rhs7(w4_s, (FH, FH, 0, 0), (0, KH, 0, KH), FH, KH, zero))
                l4 = lz('l4', lambda: [
                    jnp.concatenate([st['l4', jj][q] for jj in range(FH // 128)], axis=1)
                    for q in range(7)])
                l7 = [v[OFF[k]:OFF[k] + OC[k]].astype(BF) for v in l4]
                st['h2', k] = _join(_strassen(l7, b4, _dot, '4321065'))

            def do_o(k):
                g0, n = 2 * OFF[k], 2 * OC[k]
                bo = lz('bo', lambda: _rhs7(wo_s, *square))
                a = _join(_strassen(_bf7(_quads(rows_of('o', SB, g0, n))), bo, _dot, '0143265'))
                b = rows_of('x1', CH, g0, n) + (st['h2', k] + st['tl', k]) * GOUT
                r0 = pl.multiple_of(s0 + g0, 16)
                gl = jnp.sum(xs[pl.ds(r0, n), :].astype(F32) * gw, axis=-1, keepdims=True)
                gate = 0.5 + 0.5 * jnp.tanh(0.5 * gl)
                res = (b + gate * (a - b)).astype(BF)
                parts = 2 if k == len(OC) - 1 else 1
                m = n // parts
                for u in range(parts):
                    r = pl.multiple_of(r0 + u * m, 16)
                    os_[pl.ds(r, m), :] = res[u * m:(u + 1) * m]
                    cp(os_.at[pl.ds(r, m), :], o_hbm.at[pl.ds(r, m), :], out_sem).start()

            _run(dict(W=do_w, Q=do_q, T=do_t, Y=do_y, N=do_n, L=do_l, F=do_f, O=do_o), PHASE2)
            return 0

        jax.lax.fori_loop(0, S // TM2, p2, 0)
        return 0

    jax.lax.fori_loop(0, pl.program_id(0) + 1, main, 0)
    cp(os_, o_hbm, out_sem).wait()


def _compiler_params():
    base = dict(vmem_limit_bytes=100 * 2**20)
    try:
        return pltpu.CompilerParams(disable_bounds_checks=True,
                                    disable_semaphore_checks=True, **base)
    except TypeError:
        return pltpu.CompilerParams(**base)


@jax.jit
def pallas_gated_mix__linear_kernel_hedgehog__mixer_s_mlp__prompt_kernel(
    A_x: jax.Array,
    A_wqkv: jax.Array,
    A_w_phi: jax.Array,
    A_wo: jax.Array,
    B_x: jax.Array,
    B_w1: jax.Array,
    B_w2: jax.Array,
    B_w3: jax.Array,
    B_w4: jax.Array,
    gate_w: jax.Array,
):
    del B_x
    x = A_x.reshape(S, D)
    wphi = jnp.transpose(A_w_phi, (1, 2, 0)).reshape(DH * DH, H)
    hbm = pl.BlockSpec(memory_space=pl.ANY)
    out = pl.pallas_call(
        _kernel,
        out_shape=jax.ShapeDtypeStruct((S, D), BF),
        grid=(1,),
        in_specs=[hbm] * 9,
        out_specs=hbm,
        scratch_shapes=[
            pltpu.VMEM((S, D), BF),
            pltpu.VMEM((D, D), BF),
            pltpu.VMEM((D, D), BF),
            pltpu.VMEM((D, D), BF),
            pltpu.VMEM((DH * DH, H), BF),
            pltpu.VMEM((D, D), BF),
            pltpu.VMEM((D, D), BF),
            pltpu.VMEM((D, D), BF),
            pltpu.VMEM((F, D), BF),
            pltpu.VMEM((F, D), BF),
            pltpu.VMEM((D,), BF),
            pltpu.VMEM((S, D), BF),
            pltpu.VMEM((PR // 2, D), jnp.uint32),
            pltpu.VMEM((4, S + 16, 128), F32),
            pltpu.VMEM((G, 64, 128), BF),
            pltpu.VMEM((G, 128, 128), F32),
            pltpu.SemaphoreType.DMA((4,)),
        ],
        compiler_params=_compiler_params(),
    )(x, A_wqkv, wphi, A_wo, B_w1, B_w2, B_w3.T, B_w4, gate_w)
    return out.reshape(1, S, D)
```
